```python
import os as _os
_os.environ.setdefault('JAX_PLATFORMS', 'cpu')
import jax
import jax.numpy as jnp

def _softmax(x, axis=-1):
    return jax.nn.softmax(x, axis=axis)

def _gelu(x):
    return jax.nn.gelu(x, approximate=True)

def _silu(x):
    return jax.nn.silu(x)

def _sigmoid(x):
    return jax.nn.sigmoid(x)

def _layernorm(x, axis=-1, eps=1e-05):
    m = jnp.mean(x, axis=axis, keepdims=True)
    v = jnp.var(x, axis=axis, keepdims=True)
    return (x - m) / jnp.sqrt(v + eps)

def _scatter_add(tgt, idx, src, axis=0):
    return tgt.at[idx].add(src)

def _segment_sum(src, seg, n):
    return jax.ops.segment_sum(src, seg, n)

class _Rng:

    def __init__(self, key):
        self._k = key

    def _next(self):
        self._k, sub = jax.random.split(self._k)
        return sub

    def normal(self, shape):
        return jax.random.normal(self._next(), shape, dtype=jnp.bfloat16)

    def randint(self, lo, hi, shape):
        return jax.random.randint(self._next(), shape, lo, hi, dtype=jnp.int32)

    def uniform(self, shape, lo=0.0, hi=1.0):
        return jax.random.uniform(self._next(), shape, jnp.bfloat16, lo, hi)

    def permutation(self, n):
        return jax.random.permutation(self._next(), n)
kernel_name = 'recurrent_scan__spectral_gfnet__mixer_gmlp__prompt'

def setup_inputs():
    _rng = _Rng(jax.random.key(int.from_bytes(__import__("os").urandom(4), "little")))
    _w = lambda a: (lambda t: t.astype(jnp.bfloat16) if jnp.issubdtype(t.dtype, jnp.floating) else t)(jnp.asarray(a))

    def _A_setup():
        B, S, D = (1, 2048, 512)
        Df = D // 2 + 1
        return {'x': _w((lambda *s: _rng.normal(s) * 0.05)(B, S, D)), 'w_r': _w((lambda *s: _rng.normal(s) * 0.1)(S, Df) * 0.02), 'w_i': _w((lambda *s: _rng.normal(s) * 0.1)(S, Df) * 0.02)}
    _A_in = _A_setup()

    def _B_setup():
        B, S, D, F = (1, 2048, 512, 1376)
        Fh = F // 2
        return {'x': _w((lambda *s: _rng.normal(s) * 0.05)(B, S, D)), 'w_in': _w((lambda *s: _rng.normal(s) * 0.4)(D, 2 * Fh)), 'w_sp': _w(0.01 * (lambda *s: _rng.normal(s) * 0.4)(S, S)), 'b_sp': _w(1.0 + 0.01 * (lambda *s: _rng.normal(s) * 0.05)(S)), 'w_out': _w((lambda *s: _rng.normal(s) * 0.05)(Fh, D))}
    _B_in = _B_setup()
    return {'A_x': _A_in['x'], 'A_w_r': _A_in['w_r'], 'A_w_i': _A_in['w_i'], 'B_x': _B_in['x'], 'B_w_in': _B_in['w_in'], 'B_w_sp': _B_in['w_sp'], 'B_b_sp': _B_in['b_sp'], 'B_w_out': _B_in['w_out']}

def reference(A_x, A_w_r, A_w_i, B_x, B_w_in, B_w_sp, B_b_sp, B_w_out):

    def _A_ref(x, w_r, w_i):
        B, S, D = x.shape
        X = (lambda x, axes=(-2, -1): jnp.fft.rfft2(x.astype(jnp.float32), axes=axes))(x, axes=(-2, -1))
        W = w_r + 1j * w_i
        X = X * W
        y = (lambda x, s, axes=(-2, -1): jnp.fft.irfft2(x, s=s, axes=axes).astype(jnp.bfloat16))(X, (S, D), axes=(-2, -1))
        return y

    def _B_ref(x, w_in, w_sp, b_sp, w_out):
        B, S, D = x.shape
        F = w_in.shape[-1]
        Fh = F // 2
        z = _gelu(jnp.einsum('bsd,df->bsf', x, w_in))
        z1 = z[..., :Fh].copy()
        z2 = _layernorm(z[..., Fh:], axis=-1)
        g = jnp.einsum('ts,bsf->btf', w_sp, z2) + b_sp[None, :, None]
        return jnp.einsum('bsf,fd->bsd', z1 * g, w_out)
    x = A_x
    xn = _layernorm(x, axis=-1)
    s = _A_ref(xn, A_w_r, A_w_i)
    g = _silu(_B_ref(xn, B_w_in, B_w_sp, B_b_sp, B_w_out))
    return x + s * g
```

```python
import math

import jax
import jax.numpy as jnp
import numpy as np
import jax.experimental.pallas as pl
import jax.experimental.pallas.tpu as pltpu

S = 2048
D = 512
F = 1376
FH = 688
FHP = 768
NB = 16
NX = 528
EPS = 1e-5

_C = math.sqrt(2.0 / math.pi)
_A = 0.044715
KAPPA = (_C * _A) ** (1.0 / 3.0)
BETA = _C / KAPPA
EPS2 = 4.0 * KAPPA * KAPPA * EPS
INV4K = 1.0 / (4.0 * KAPPA)

_NT = (((1,), (1,)), ((), ()))
_NN = (((1,), (0,)), ((), ()))
_TN = (((0,), (0,)), ((), ()))


def _pack_rows(m):
    u = np.ascontiguousarray(m, dtype=np.float32).view(np.uint32).astype(np.uint64)
    b = ((u + 0x7FFF + ((u >> 16) & 1)) >> 16).astype(np.uint32)
    return b[0::2] | (b[1::2] << 16)


def _tables():
    n2 = np.arange(128)
    gf = np.zeros((4, 128, 256))
    mi = np.zeros((4, 128, 256))
    for c in range(4):
        for j in range(64):
            k = 4 * j + c
            th = 2 * np.pi * k * n2 / 512
            co, si = np.cos(th), np.sin(th)
            m, r = j // 8, j % 8
            re = 16 * m + r
            im = re + 8
            kre = 16 * m + 2 * r
            kim = kre + 1
            w = 1.0 if k == 0 else 2.0
            if c in (0, 2):
                gf[c, re, :128], gf[c, im, :128] = co, -si
                mi[c, kre, :128], mi[c, kim, :128] = w * co, -w * si
            elif c == 1:
                gf[c, re, :128], gf[c, re, 128:] = co, -si
                gf[c, im, :128], gf[c, im, 128:] = -si, -co
                mi[c, kre, :128], mi[c, kim, :128] = w * co, -w * si
                mi[c, kre, 128:], mi[c, kim, 128:] = -w * si, -w * co
            else:
                gf[c, re, :128], gf[c, re, 128:] = co, si
                gf[c, im, :128], gf[c, im, 128:] = -si, co
                mi[c, kre, :128], mi[c, kim, :128] = w * co, -w * si
                mi[c, kre, 128:], mi[c, kim, 128:] = w * si, w * co
    nyq = np.cos(np.pi * n2)
    g0 = np.zeros((144, 128))
    g0[:128] = gf[0, :, :128]
    g0[128:136] = nyq
    g2 = np.zeros((144, 128))
    g2[:128] = gf[2, :, :128]
    mi[0, 1, :128] = nyq
    godd = np.zeros((256, 256))
    for n, c in enumerate((1, 3)):
        ks = 4 * np.arange(64) + c
        th = 2 * np.pi * np.outer(ks, n2) / 512
        godd[64 * n:64 * n + 64, :128] = np.cos(th) - np.sin(th)
        godd[64 * n:64 * n + 64, 128:] = (np.cos(th) + np.sin(th)) * (-1.0 if c == 1 else 1.0)
        godd[128:192, 128 * n:128 * n + 128] = np.cos(th)
    fs = 1.0 / KAPPA
    bs = 1.0 / (S * D)
    cc = np.cos(2 * np.pi * np.outer(n2, n2) / 128)
    ss = np.sin(2 * np.pi * np.outer(n2, n2) / 128)
    cb = np.concatenate(
        [
            godd * fs,
            np.concatenate([g0, g2], 1) * fs,
            mi[1] * bs,
            mi[3] * bs,
            np.concatenate([mi[0, :, :128], mi[2, :, :128]], 1) * bs,
            np.concatenate([cc, np.zeros((128, 128))], 1),
            np.concatenate([ss - cc, -ss - cc], 1),
        ],
        0,
    )
    k1 = np.arange(16)
    ph = 2 * np.pi * np.outer(k1, n2) / 2048
    tw = np.concatenate([np.cos(ph), np.sin(ph)], 1)
    tw = np.repeat(tw, 8, axis=0).astype(np.float32)
    return _pack_rows(cb), tw


_CB, _TW = _tables()


def _bf(u32):
    return pltpu.bitcast(u32, jnp.bfloat16)


def _u32(bf):
    return pltpu.bitcast(bf, jnp.uint32)


def _bits(f):
    return jax.lax.bitcast_convert_type(f, jnp.uint32)


def _dot(a, b, dims):
    return jax.lax.dot_general(a, b, dims, preferred_element_type=jnp.float32)


def _pk2(a, b):
    return pltpu.pack_elementwise([a, b], packed_dtype=jnp.bfloat16)


def _pk(v):
    n = v.shape[0] // 16
    v3 = v.reshape(n, 16, 128)
    return _pk2(v3[:, 0:8, :], v3[:, 8:16, :]).reshape(8 * n, 128)


def _unpk(u):
    lo = jax.lax.bitcast_convert_type(u << 16, jnp.float32)
    hi = jax.lax.bitcast_convert_type(u & jnp.uint32(0xFFFF0000), jnp.float32)
    return lo, hi


def _radix4(a, sign):
    (ar, ai), (br, bi), (cr, ci), (dr, di) = a
    s0r, s0i = ar + cr, ai + ci
    d0r, d0i = ar - cr, ai - ci
    s1r, s1i = br + dr, bi + di
    d1r, d1i = br - dr, bi - di
    o0 = (s0r + s1r, s0i + s1i)
    o2 = (s0r - s1r, s0i - s1i)
    if sign < 0:
        o1 = (d0r + d1i, d0i - d1r)
        o3 = (d0r - d1i, d0i + d1r)
    else:
        o1 = (d0r - d1i, d0i + d1r)
        o3 = (d0r + d1i, d0i - d1r)
    return [o0, o1, o2, o3]


def _tw16(x, e, sign):
    e = e % 16
    xr, xi = x
    if e == 0:
        return x
    if e == 4:
        return (xi, -xr) if sign < 0 else (-xi, xr)
    if e in (2, 6):
        h = math.sqrt(0.5)
        if e == 2:
            if sign < 0:
                return ((xr + xi) * h, (xi - xr) * h)
            return ((xr - xi) * h, (xi + xr) * h)
        if sign < 0:
            return ((xi - xr) * h, (xr + xi) * (-h))
        return ((xr + xi) * (-h), (xr - xi) * h)
    ang = sign * 2 * math.pi * e / 16
    wr, wi = math.cos(ang), math.sin(ang)
    return (xr * wr - xi * wi, xr * wi + xi * wr)


def _fft16_a(a4, n0, sign):
    o = _radix4(a4, sign)
    return [_tw16(o[k0], n0 * k0, sign) for k0 in range(4)]


MH = 352
MQ = 176
KQ = S // 4
SYL = 144

CFG = dict(
    q0=dict(wo=[1, 7], wa=[8, 21], wb=[22, 48], s1=[8, 20], f=28, i=31, s3=[34, 44]),
    tf=[5, 14, 23, 32], fs=[[0, 4, 10, 13], [6, 9, 19, 22], [15, 18, 28, 36], [24, 27, 39, 48]],
    lnw=34, lnb=8, win=8, tz2=[0, 0, 8, 16], tz1=[6, 6, 6, 6, 0, 0, 0],
)


def _str_l(a11, a12, a21, a22):
    return (a11 + a22, a21 + a22, a11, a21 - a11, a11 + a12, a22, a12 - a22)


def _str_r(b11, b21, b12, b22):
    return (b11 + b22, b11, b12 - b22, b11 + b12, b22, b21 - b11, b21 + b22)


_RDIR = {1: (0, 0), 4: (1, 1)}


def _kernel(
    x_hbm, wr_hbm, wi_hbm, win_hbm, wsp_hbm, b_hbm, wout_hbm, cb_hbm, tw_hbm, z_hbm,
    o_hbm,
    xb, winb, wint, woutb, woutp, wspb, bb, bbc, wrb, wib, w32r, w32i, w32n, wtr, wti,
    cb, tw, xs0, xs1, wz, qa, qb, qc, qd, qe, qf, qg, qh, qi, qj, ys0, ys1, ys2, ys3, ls0, ls1, st_m, st_r,
    x1, y1s, zf0, zf1, zf2, zf3, xa0, xa1, sa, tbx, tby, ua, ub, uc, ud, ue, uf, ug, va, vb, vc, vd, ve, vf, vg,
    h0, h1, h2, h3, lf, li, do, nyb, yp, gate, sbuf, ob, zs, sems,
):
    f32, u32 = jnp.float32, jnp.uint32
    nsem = [0]

    def cp(src, dst):
        return pltpu.make_async_copy(src, dst, sems.at[nsem[0]])

    def group(*cps):
        nsem[0] += 1
        return [c for x in cps for c in (x if isinstance(x, list) else [x])]

    def rows(ref, lo, hi):
        return ref.at[pl.ds(lo, hi - lo), :]

    def xcp(lo, hi):
        return cp(x_hbm.at[0, pl.ds(lo * 128, (hi - lo) * 128), :], rows(xb, lo * 128, hi * 128))

    def wspcp(lo, hi):
        return [cp(rows(wsp_hbm, h + lo, h + hi), rows(wspb, h + lo, h + hi)) for h in (0, KQ, 2 * KQ, 3 * KQ)]

    def o_cp(lo, hi):
        return cp(rows(ob, lo * 128, hi * 128), o_hbm.at[0, pl.ds(lo * 128, (hi - lo) * 128), :])

    grp_z = group(cp(z_hbm, zs))
    grp_a = group(xcp(0, 1))
    grp_b = group(xcp(8, 9), cp(rows(win_hbm, FH, FH + MH), rows(winb, FH, FH + MH)))
    grp_c = group(cp(rows(win_hbm, FH + MH, F), rows(winb, FH + MH, F)), xcp(4, 5), xcp(12, 13))
    grp_d = group(cp(rows(win_hbm, 0, FH), rows(winb, 0, FH)), cp(rows(cb_hbm, 0, 200), rows(cb, 0, 200)),
                  xcp(1, 2), xcp(9, 10))
    grp_1 = group(xcp(5, 6), xcp(13, 14), xcp(2, 3), xcp(10, 11), wspcp(0, 48))
    grp_2 = group(xcp(6, 8), xcp(14, 16), xcp(3, 4), xcp(11, 12), wspcp(48, 128))
    grp_3 = group(wspcp(128, 256), cp(wr_hbm, wrb), cp(wi_hbm, wib), cp(wout_hbm, woutb),
                  cp(rows(cb_hbm, 200, 520), rows(cb, 200, 520)), cp(tw_hbm, tw))
    grp_3 += group(cp(b_hbm, bb.at[pl.ds(0, S)]))
    grp_4 = group(wspcp(256, 512))

    def wait(grp):
        for c_ in grp:
            c_.wait()

    for c_ in grp_z + grp_a + grp_b + grp_c + grp_d + grp_1 + grp_2 + grp_3 + grp_4:
        c_.start()
    wait(grp_z + grp_a)

    zr = [zs[n] for n in range(3)]
    zvec = jnp.full((8, 128), zr[2], jnp.int32).astype(u32)

    def dyn(lo, n, w=0, stride=None):
        if stride is None:
            return pl.ds(pl.multiple_of(zr[w] + lo, 8), n)
        return pl.ds(zr[w] + lo, n, stride=stride)

    def blk(i, n, extra=0):
        if isinstance(i, int):
            return i * n + extra
        return pl.multiple_of(i * n + extra, 8)

    def token(*vs):
        acc = None
        for v in vs:
            if v.dtype != u32:
                v = _bits(v)
            for r in range(0, v.shape[0], 8):
                for c in range(0, v.shape[1], 128):
                    t = v[r:r + 8, c:c + 128]
                    acc = t if acc is None else acc | t
        return acc

    sync = [None]

    def synced(u):
        if sync[0] is None:
            return u
        sz = sync[0] & zvec
        cols = [u[0:8, c:c + 128] | sz for c in range(0, u.shape[1], 128)]
        return jnp.concatenate([jnp.concatenate(cols, axis=1), u[8:]], axis=0)

    def tiev(v, toks):
        parts = []
        prev = 0
        for r in sorted(toks):
            if r * 8 > prev:
                parts.append(v[prev:r * 8])
            parts.append(jax.lax.bitcast_convert_type(_bits(v[r * 8:r * 8 + 8]) | (toks[r] & zvec), f32))
            prev = r * 8 + 8
        if prev < v.shape[0]:
            parts.append(v[prev:])
        return jnp.concatenate(parts, axis=0) if len(parts) > 1 else parts[0]

    ALL = 9999
    rel = [None]

    def gate_(v):
        if rel[0] is None:
            return v
        u = v if v.dtype == u32 else _bits(v)
        tiles = [[u[r:r + 8, c:c + 128] | rel[0] for c in range(0, u.shape[1], 128)]
                 for r in range(0, u.shape[0], 8)]
        u = jnp.concatenate([jnp.concatenate(t, axis=1) for t in tiles], axis=0)
        return u if v.dtype == u32 else jax.lax.bitcast_convert_type(u, v.dtype)

    class Job:
        def __init__(self, gen, n, win=None):
            self.gen, self.left, self.win = gen, n, CFG["win"] if win is None else win

        def __next__(self):
            self.left -= 1
            return next(self.gen)

    def spread(lists, nslot, src=None):
        out = {}
        rels = {}
        for job, n, lo, hi in lists:
            n = min(n, job.left)
            for k in range(n):
                sl = min(int(nslot * (lo + (k + 0.5) * (hi - lo) / n)), nslot - 1)
                rs = sl - job.win
                if src is not None and rs >= 0:
                    if rs not in rels:
                        rels[rs] = _bits(src[8 * rs:8 * rs + 8]) & zvec
                    rel[0] = rels[rs]
                tk = next(job)
                rel[0] = None
                out[sl] = tk if sl not in out else out[sl] | tk
        return out

    def add(d, k, v):
        d.setdefault(k, []).append(v)

    def over(jobs, job, lo, hi):
        n = -(-job.left // (hi - lo))
        for pos in range(lo, hi):
            add(jobs, pos, (job, n if pos < hi - 1 else ALL, 0.0, 1.0))

    xsb, ysb, zfb = (xs0, xs1), (ys0, ys1, ys2, ys3), (zf0, zf1, zf2, zf3)
    TOFF = (0, 8, 4, 12)
    row8 = jax.lax.broadcasted_iota(jnp.int32, (8, 128), 0)

    def ln_stats(x):
        m = jnp.sum(x, axis=-1, keepdims=True) * (1.0 / D)
        v = jnp.sum(x * x, axis=-1, keepdims=True) * (1.0 / D) - m * m
        return m, jax.lax.rsqrt(jnp.maximum(v, 0.0) + EPS) * KAPPA

    def xrows(i, r):
        return _unpk(gate_(_u32(xb[pl.ds(blk(i, 128, r), 16), :])))

    def lns_job(i, p):
        def gen():
            for r in range(0, 128, 16):
                for e in range(2):
                    st = [jnp.broadcast_to(v, (8, 128)) for x in xrows(i + 8 * e, r) for v in ln_stats(x)]
                    for n, v in enumerate(st):
                        (ls1 if p else ls0)[e, 2 * r + 8 * n:2 * r + 8 * n + 8, :] = v
                    yield token(*st)
        return Job(gen(), 16, CFG["lnw"])

    def ln_rows(i, b, r, pre=False):
        outs = []
        for e, x in enumerate(xrows(i, r)):
            if pre:
                ls = ls1 if b // 2 else ls0
                m, rs = (ls[b % 2, dyn(2 * r + 16 * e + 8 * n, 8), :] for n in range(2))
                a0, a1, a2, a3 = ((x[:, 128 * j:128 * (j + 1)] - m) * rs for j in range(4))
                xn = jnp.concatenate([a0, a1, a2, a3], axis=1)
            else:
                m, rs = ln_stats(x)
                xn = (x - m) * rs
                a0, a1, a2, a3 = (xn[:, 128 * j:128 * (j + 1)] for j in range(4))
            s02, s13 = a0 + a2, a1 + a3
            p, q = a0 - a2, a1 - a3
            outs.append((xn, jnp.concatenate([s02 + s13, s02 - s13, p, q, p + q, p - q], axis=1)))
        py = _pk2(outs[0][1], outs[1][1])
        ysb[b][r // 2:r // 2 + 8, :] = py
        px = _pk2(outs[0][0], outs[1][0])
        for hf in range(2):
            xsb[b // 2][PLAIN[b % 2][hf], r // 2:r // 2 + 8, :] = px[:, 256 * hf:256 * (hf + 1)]
        return outs[0][0], outs[1][0], token(px, py)

    PLAIN = ((1, 7), (8, 4))

    def ln_job(i, b):
        def gen():
            for r in range(0, 128, 16):
                yield ln_rows(i, b, r)[2]
        return Job(gen(), 8, CFG["lnw"])

    def lnp_job(i, p, win=None, pre=True):
        def gen():
            for r in range(0, 128, 16):
                a = ln_rows(i, 2 * p, r, pre)
                yield a[2]
                b = ln_rows(i + 8, 2 * p + 1, r, pre)
                ops = [_str_r(a[e][:, 0:256], a[e][:, 256:512], b[e][:, 0:256], b[e][:, 256:512])
                       for e in range(2)]
                pks = []
                for n in range(7):
                    if n not in _RDIR:
                        pks.append(_pk2(ops[0][n], ops[1][n]))
                        xsb[p][n, r // 2:r // 2 + 8, :] = pks[-1]
                yield token(b[2], *pks)
        return Job(gen(), 16, CFG["lnw"] if win is None else win)

    def wz_job():
        def ld(r, lanes):
            if r >= FH:
                return (jnp.zeros((8, 128), f32),) * 2
            v = gate_(winb[r:r + 16, lanes].astype(f32))
            return v[0:8], v[8:16]

        def gen():
            for r in range(0, MH, 16):
                for c in range(2):
                    lo, hi = slice(c * 128, (c + 1) * 128), slice(256 + c * 128, 256 + (c + 1) * 128)
                    a = [ld(r, lo), ld(r, hi), ld(MH + r, lo), ld(MH + r, hi)]
                    ops = [_str_l(*[v[e] for v in a]) for e in range(2)]
                    pks = [_pk2(ops[0][n], ops[1][n]) for n in range(7)]
                    for n in range(7):
                        wz[n, r // 2:r // 2 + 8, lo] = pks[n]
                    yield token(*pks)
        return Job(gen(), 44)

    def gelu2(z):
        return z + z * jnp.tanh(z * (z * z + BETA))

    def cdot(r0, r1, lanes, w):
        outs = []
        r = r0
        while r < r1:
            n = min(64, r1 - r)
            if r1 - r - n == 16:
                n += 16
            outs.append(_dot(_bf(cb[r // 2:(r + n) // 2, lanes]), w, _NT))
            r += n
        return jnp.concatenate(outs, axis=0)

    L0, L1 = slice(0, 128), slice(128, 256)

    def l1_job(kq):
        xa = xa1 if kq else xa0
        G = 32

        def nrm(e, lo, n, mg):
            z = zfb[2 * kq + e][dyn(lo, n, 1), :].reshape(n // 8, 8, 128)
            return ((z - mg[e]) * st_r[dyn(8 * (2 * kq + e), 8), :]).reshape(n, 128)

        def gen():
            for r in range(0, MH, G):
                n2 = min(G, FH - MH - r)
                mg = [gate_(st_m[dyn(8 * (2 * kq + e), 8), :]) for e in range(2)]
                top = [nrm(e, r, G, mg) for e in range(2)]
                bot = [nrm(e, MH + r, n2, mg) for e in range(2)]
                if n2 < G:
                    pad = jnp.zeros((G - n2, 128), f32)
                    bot = [jnp.concatenate([v, pad], axis=0) for v in bot]
                ops = _str_l(top[0], top[1], bot[0], bot[1])
                for n, v in enumerate(ops):
                    xa[n, r:r + G, :] = v
                yield token(*[ops[n] for n in (0, 1, 3, 4, 6)])
        return Job(gen(), 11)

    def l2_job(kt):
        def gen():
            G = 16
            for n in range(7):
                for r in range(0, MQ, G):
                    ops = _str_l(gate_(xa0[n, dyn(r, G), :]), xa1[n, dyn(r, G), :],
                                 xa0[n, dyn(MQ + r, G), :], gate_(xa1[n, dyn(MQ + r, G), :]))
                    pks = [_pk(v) for v in ops]
                    for m, v in enumerate(pks):
                        sa[kt, 7 * n + m, r // 2:(r + G) // 2, :] = v
                    yield token(*pks)
        return Job(gen(), 77)

    def wprep_a_job():
        def gen():
            for b in range(NB):
                lanes = slice(b * 128, (b + 1) * 128)
                rws = slice(64 * b, 64 * (b + 1))
                for src, w32 in ((wrb, w32r), (wib, w32i)):
                    for j in range(2):
                        v = _u32(src[j * 128:(j + 1) * 128, lanes].T)
                        w32[j, rws, :] = v
                        yield token(v)
                nr, ni = (jnp.broadcast_to(src[256:257, lanes].astype(f32), (8, 128)) for src in (wrb, wib))
                ny = jnp.where(row8 == 0, nr, jnp.where(row8 == 4, ni, 0.0))
                slab = jnp.concatenate([_pk2(ny, jnp.zeros((8, 128), f32)), jnp.zeros((56, 128), u32)], axis=0)
                v = _u32(_bf(slab).T)
                w32n[rws, :] = v
                yield token(v)
        return Job(gen(), 80)

    def wprep_b_job():
        def gen():
            for r0 in range(8):
                tt = w32n[dyn(r0, 128, 0, 8), :].T[0:16]
                wtr[0, 256 + r0:257 + r0, :] = tt[0:1]
                wti[0, 256 + r0:257 + r0, :] = tt[8:9]
                yield token(tt)
            for r0 in range(8):
                for w32, wt in ((w32r, wtr), (w32i, wti)):
                    for j in range(2):
                        tt = w32[j, dyn(r0, 128, 0, 8), :].T
                        wt[r0, j * 128:(j + 1) * 128, :] = tt
                        yield token(tt)
        return Job(gen(), 40)

    def wout_job():
        def gen():
            woutp[FH // 2:FHP // 2, :] = jnp.zeros(((FHP - FH) // 2, D), u32)
            bvec = (bb[0:S].astype(f32) * INV4K).reshape(1, S)
            for j in range(NB):
                bbc[j, 0:8, :] = jnp.broadcast_to(bvec[:, j * 128:(j + 1) * 128], (8, 128))
            for c in range(4):
                lanes = slice(c * 128, (c + 1) * 128)
                for lo in range(0, FH, 64):
                    hi = min(lo + 64, FH)
                    w1 = _bf(_pk(woutb[lo:hi, lanes].astype(f32)))
                    v = _pk(w1.astype(f32))
                    woutp[lo // 2:hi // 2, lanes] = v
                    yield token(v)
        return Job(gen(), 44)

    def tslot(n, m):
        return (tbx, 7 * n + m) if n < 4 else (tby, 7 * (n - 4) + m)

    def tprep_job(q, part, r_lo=0, nr=8):
        def gen():
            for rr in range(nr):
                r = r_lo + rr
                if not isinstance(r, int):
                    r = jnp.minimum(r, 7)
                ro = pl.ds(blk(r, 8), 8)
                for c in range(4):
                    lanes = slice(c * 128, (c + 1) * 128)

                    def up(tn, kq):
                        base = blk(q, 128, tn * KQ) + blk(r, 16)
                        if not isinstance(base, int):
                            base = pl.multiple_of(base, 16)
                        return _unpk(gate_(_u32(wspb[pl.ds(base, 16), kq * KQ + c * 128:kq * KQ + (c + 1) * 128])))

                    def level2(n, y):
                        ops = [_str_r(y[0, 0][h], y[1, 0][h], y[0, 1][h], y[1, 1][h]) for h in range(2)]
                        pks = []
                        for m in range(7):
                            if n in _RDIR and m in _RDIR:
                                continue
                            pks.append(_pk2(ops[0][m], ops[1][m]))
                            t, ix = tslot(n, m)
                            t[ix, ro, lanes] = pks[-1]
                        return token(*pks)

                    def cmb(a, b, sg):
                        if sg > 0:
                            return {k: (a[k][0] + b[k][0], a[k][1] + b[k][1]) for k in a}
                        return {k: (a[k][0] - b[k][0], a[k][1] - b[k][1]) for k in a}

                    def blk4(tn0, kq0):
                        return {(kq, tn): up(tn0 + tn, kq0 + kq) for kq in range(2) for tn in range(2)}

                    if part == 0:
                        b11 = blk4(0, 0)
                        yield level2(1, b11)
                        b22 = blk4(2, 2)
                        yield level2(0, cmb(b11, b22, 1))
                        b12 = blk4(2, 0)
                        yield level2(2, cmb(b12, b22, -1))
                        yield level2(3, cmb(b11, b12, 1))
                    else:
                        b22 = blk4(2, 2)
                        yield level2(4, b22)
                        b21 = blk4(0, 2)
                        yield level2(6, cmb(b21, b22, 1))
                        yield level2(5, cmb(b21, blk4(0, 0), -1))
        return Job(gen(), nr * 4 * (4 - part))

    def xplain(b, w):
        return _bf(jnp.concatenate([xsb[b // 2][n, dyn(0, 64, w), :] for n in PLAIN[b % 2]], axis=1))

    def z2_sink(b, lo, z, tk, st):
        CH = 4
        ng = z.shape[0] // 8
        marks = []
        for r in range(0, ng, CH):
            n = min(CH, ng - r)
            tkc = {k - r: v for k, v in tk.items() if r <= k < r + n}
            if len(marks) >= 2:
                tkc[0] = marks[-2] if 0 not in tkc else tkc[0] | marks[-2]
            y = gelu2(tiev(z[8 * r:8 * (r + n)], tkc))
            zfb[b][lo + 8 * r:lo + 8 * (r + n), :] = y
            for q in range(n):
                if "c" not in st:
                    st["c"] = y[0:8]
                    continue
                d = y[8 * q:8 * q + 8] - st["c"]
                st["sm"] = d if "sm" not in st else st["sm"] + d
                st["sq"] = d * d if "sq" not in st else st["sq"] + d * d
            marks.append(token(st["sm"], st["sq"]))
        st["n"] = st.get("n", 0) + ng
        if st["n"] == FH // 8:
            c, sm, sq, cnt = st["c"], st["sm"], st["sq"], FH // 8
            m2 = jnp.sum(sm + cnt * c, axis=0, keepdims=True) * (1.0 / FH)
            e = m2 - c
            v2 = jnp.sum(sq - 2.0 * e * sm + cnt * (e * e), axis=0, keepdims=True) * (1.0 / FH)
            st_m[8 * b:8 * b + 8, :] = jnp.broadcast_to(m2, (8, 128))
            st_r[8 * b:8 * b + 8, :] = jnp.broadcast_to(
                jax.lax.rsqrt(jnp.maximum(v2, 0.0) + EPS2) * INV4K, (8, 128))

    def z2_op(b, la, gated=True):
        z = _dot(_bf(wint[dyn(0, FH // 2), :]), xplain(b, 0), _NT)
        z2_sink(b, 0, z, spread(la, 86, z if gated else None), {})

    dq0, dq1 = dyn(0, MH, 0), dyn(0, MH, 1)

    def z1_chains(kt, jobs):
        rnd = [0]
        tks = []

        def pr(p, n):
            return _dot(_bf(synced(wz[n, dyn(0, MH // 2), :])), _bf(xsb[p][n, dyn(0, 64, 1), :]), _NT)

        def two(a, b):
            ra, rb = pr(*a), pr(*b)
            tks[:] = [spread(jobs.get(rnd[0], []), 42, ra)]
            sync[0] = token(ra[MH - SYL:MH - SYL + 8], rb[MH - SYL:MH - SYL + 8])
            rnd[0] += 1
            return ra, rb

        def tie1(v):
            return tiev(v, tks.pop()) if tks else v

        def out(b, lo, v):
            v = v[0:min(MH, FH - lo)]
            y1s[kt + TOFF[b], lo:lo + v.shape[0], :] = tie1(v)

        m1, m2 = two((0, 0), (0, 1))
        qa[...] = tie1(m1)
        qb[...] = m2
        qc[...] = m1 - m2
        m3, m6 = two((0, 2), (0, 3))
        out(1, MH, qc[dq0, :] + m3 + m6)
        qd[...] = m3
        m5, m4 = two((0, 4), (0, 5))
        out(1, 0, qd[dq0, :] + m5)
        out(0, MH, qb[dq0, :] + m4)
        qe[...] = qa[dq0, :] + m4 - m5
        m7, m1 = two((0, 6), (1, 0))
        out(0, 0, qe[dq0, :] + m7)
        qf[...] = m1
        m2, m3 = two((1, 1), (1, 2))
        qg[...] = tie1(m2)
        qh[...] = m3
        qi[...] = qf[dq0, :] - m2 + m3
        m6, m5 = two((1, 3), (1, 4))
        out(3, MH, qi[dq0, :] + m6)
        out(3, 0, qh[dq0, :] + m5)
        qj[...] = qf[dq1, :] - m5
        m4, m7 = two((1, 5), (1, 6))
        out(2, MH, qg[dq0, :] + m4)
        out(2, 0, qj[dq0, :] + m4 + m7)

    def d_op(i, b):
        y0, y2, p, q, pp, pm = (_bf(ysb[b][dyn(0, 64), 128 * n:128 * (n + 1)]) for n in range(6))
        o0 = cdot(256, 400, L0, y0)
        x1[i, 0:128, :] = o0[0:128]
        x1[i, 512:520, :] = o0[128:136]
        x1[i, 256:384, :] = cdot(256, 384, L1, y2)
        for n, (base, w) in enumerate(((128, pp), (384, pm))):
            t = cdot(128, 192, (L0, L1)[n], w)
            re = t + cdot(64 * n, 64 * n + 64, L1, q)
            im = cdot(64 * n, 64 * n + 64, L0, p) - t
            for m in range(8):
                x1[i, base + 16 * m:base + 16 * m + 8, :] = re[8 * m:8 * m + 8]
                x1[i, base + 16 * m + 8:base + 16 * m + 16, :] = im[8 * m:8 * m + 8]

    def p1_start():
        sts = [{}, {}]

        def z2_part(b, lo, hi, la):
            if b == 0:
                cols = []
                for c in range(4):
                    lanes = slice(c * 128, (c + 1) * 128)
                    cols.append(_u32(winb[FH + lo:FH + hi, lanes]))
                    wint[lo // 2:hi // 2, lanes] = cols[-1]
                lhs = jnp.concatenate(cols, axis=1)
            else:
                lhs = wint[dyn(lo // 2, (hi - lo) // 2), :]
            z = _dot(_bf(lhs), xplain(b, lo // MH), _NT)
            z2_sink(b, lo, z, spread(la, (hi - lo) // 8), sts[b])

        def z1_op(b, lb):
            if b == 0:
                cols = []
                for c in range(4):
                    lanes = slice(c * 128, (c + 1) * 128)
                    cols.append(_pk(winb[0:FH, lanes].astype(f32)))
                    wint[FH // 2:FH, lanes] = cols[-1]
                lhs = jnp.concatenate(cols, axis=1)
            else:
                lhs = wint[dyn(FH // 2, FH // 2), :]
            z = _dot(_bf(lhs), xplain(b, 1), _NT)
            y1s[TOFF[b], 0:FH, :] = tiev(z, spread(lb, 86, z))
            d_op(TOFF[b], b)

        lnj = ln_job(0, 0)
        while lnj.left:
            next(lnj)
        wait(grp_b)
        z2_part(0, 0, MH, [(ln_job(8, 1), ALL, 0.0, 0.6)])
        z2_part(1, 0, MH, [])
        wait(grp_c)
        ln4 = ln_job(4, 2)
        z2_part(0, MH, FH, [(ln4, 5, 0.0, 1.0)])
        z2_part(1, MH, FH, [(ln4, ALL, 0.0, 0.5)])
        z2_op(2, [(ln_job(12, 3), ALL, 0.0, 0.7)])
        z2_op(3, [(l1_job(0), ALL, 0.2, 1.0)])
        wait(grp_d)
        wzj, l2j, lnj = wz_job(), l2_job(0), lnp_job(1, 0, None, False)
        z1_op(0, [(l1_job(1), ALL, 0.0, 1.0), (wzj, 15, 0.0, 1.0)])
        z1_op(1, [(l2j, 30, 0.1, 1.0), (wzj, ALL, 0.0, 1.0)])
        z1_op(2, [(lnj, 8, 0.0, 1.0), (l2j, 25, 0.0, 1.0)])
        z1_op(3, [(lnj, ALL, 0.0, 0.8), (l2j, ALL, 0.0, 1.0)])

    def p1_quad(kt, bg):
        nk = jnp.minimum(kt + 1, 3)
        tz = CFG["tz2"]
        lnj = lnp_job(kt + 4, 1, CFG["lnb"])
        z2_op(0, [(lns_job(kt + 4, 1), ALL, 0.0, 0.6), (lnj, 3, 0.75, 1.0), (bg, tz[0], 0.0, 1.0)])
        z2_op(1, [(lnj, ALL, 0.0, 0.8), (bg, tz[1], 0.0, 1.0)])
        z2_op(2, [(bg, tz[2], 0.0, 1.0), (l1_job(0), ALL, 0.2, 1.0)])
        z2_op(3, [(bg, tz[3], 0.0, 1.0)])
        d_op(kt, 0)
        d_op(kt + 8, 1)
        jobs = {}
        over(jobs, l1_job(1), 0, 2)
        over(jobs, l2_job(kt), 2, 7)
        over(jobs, lns_job(nk, 0), 0, 4)
        over(jobs, lnp_job(nk, 0, CFG['lnb']), 4, 7)
        for rn, n in enumerate(CFG["tz1"]):
            add(jobs, rn, (bg, n, 0.0, 1.0))
        z1_chains(kt, jobs)
        assert bg.left == 0
        d_op(kt + 4, 2)
        d_op(kt + 12, 3)

    p1_start()
    wait(grp_1)

    def p1_body(it, carry):
        @pl.when(it == 1)
        def _():
            wait(grp_2)

        sync[0] = None
        p1_quad(1 + it, tprep_job(0, 0, 3 * it, 3))
        return carry

    jax.lax.fori_loop(0, 3, p1_body, 0)
    sync[0] = None
    wait(grp_3)

    hbufs = (h0, h1, h2, h3)

    def o_tile(q, tn, fused):
        rs = pl.ds(blk(q, 128, tn * KQ), 128)
        hp = jnp.concatenate([hbufs[tn][dyn(0, FH // 2), :], jnp.zeros(((FHP - FH) // 2, 128), u32)], axis=0)
        w = _dot(_bf(hp), _bf(woutp[dyn(0, FHP // 2), :]), _TN)
        g = w + w * jnp.tanh(w)
        sync[0] = None
        if fused:
            ob[rs, :] = (xb[rs, :].astype(f32) + sbuf[tn, dyn(0, 128), :] * g).astype(jnp.bfloat16)
        else:
            gate[rs, :] = g

    def ngr(pair):
        return sum(g is not None for g in pair)

    def lf_row(ch, gp, gi, pr):
        return sum(64 * ngr(p) for p in ch[:gp]) + (pr * ngr(ch[gp]) + gi) * 8

    def twid(k, re, im, sign):
        if k == 0:
            return re, im
        c = tw[8 * k:8 * k + 8, 0:128]
        s = tw[8 * k:8 * k + 8, 128:256]
        if sign < 0:
            return re * c + im * s, im * c - re * s
        return re * c - im * s, im * c + re * s

    def s1_job(ch, it):
        def gen():
            for gp, pair in enumerate(ch):
                for gi, g in enumerate(pair):
                    if g is None:
                        continue
                    t = []
                    for n0 in range(4):
                        a4 = [(x1[4 * n1 + n0, dyn(64 * it + 16 * g, 8), :],
                               x1[4 * n1 + n0, dyn(64 * it + 16 * g + 8, 8), :]) for n1 in range(4)]
                        t.append(_fft16_a(a4, n0, -1))
                        yield token(t[-1][1][0], t[-1][3][1], t[-1][0][0], t[-1][2][1])
                    for kp in range(2):
                        oa = _radix4([t[n0][2 * kp] for n0 in range(4)], -1)
                        ob_ = _radix4([t[n0][2 * kp + 1] for n0 in range(4)], -1)
                        for k1 in range(4):
                            k = 4 * k1 + 2 * kp
                            ar, ai = twid(k, oa[k1][0], oa[k1][1], -1)
                            br, bi = twid(k + 1, ob_[k1][0], ob_[k1][1], -1)
                            tri = (_pk2(ar + ai, br + bi), _pk2(ai, bi), _pk2(ar, br))
                            r0 = lf_row(ch, gp, gi, k // 2)
                            for n in range(3):
                                lf[n, r0:r0 + 8, :] = tri[n]
                            yield token(*tri)
        return Job(gen(), 12 * sum(ngr(p) for p in ch))

    def cdft(src, nrow, swap):
        m1 = _bf(cb[392:456, 0:128])
        m2 = _bf(cb[456:520, 0:128])
        m3 = _bf(cb[456:520, 128:256])
        if swap:
            m2, m3 = m3, m2
        nu = 4 if nrow >= 256 else (2 if nrow >= 128 else 1)
        n = nrow // nu
        for c in range(nu):
            t1 = _dot(_bf(src[0, dyn(c * n, n), :]), m1, _NN)
            yield (t1 + _dot(_bf(src[1, dyn(c * n, n), :]), m2, _NN),
                   t1 + _dot(_bf(src[2, dyn(c * n, n), :]), m3, _NN))

    def f_op(ch, it):
        zero = jnp.zeros((8, 128), f32)
        parts = list(cdft(lf, sum(64 * ngr(p) for p in ch), False))
        xr_ = jnp.concatenate([p[0] for p in parts], axis=0)
        xi_ = jnp.concatenate([p[1] for p in parts], axis=0)
        sync[0] = None
        for gp, pair in enumerate(ch):
            for pr in range(8):
                ys = []
                for gi, g in enumerate(pair):
                    if g is None:
                        ys.append([(zero, zero)] * 2)
                        continue
                    r0 = 2 * lf_row(ch, gp, gi, pr)
                    rws = dyn(256, 8) if g == 32 else dyn(32 * (g % 8) + g // 8 + 128 * it, 8, 0, 4)
                    wr_ = _bf(wtr[pr, rws, :]).astype(f32)
                    wi_ = _bf(wti[pr, rws, :]).astype(f32)
                    xr, xi = xr_[r0:r0 + 16], xi_[r0:r0 + 16]
                    yr, yi = xr * wr_ - xi * wi_, xr * wi_ + xi * wr_
                    ys.append([(yr[0:8], yi[0:8]), (yr[8:16], yi[8:16])])
                for v in range(2):
                    (ar, ai), (br, bi) = ys[0][v], ys[1][v]
                    o = gp * 128 + pr * 16 + v * 8
                    li[0, o:o + 8, :] = _pk2(ar + ai, br + bi)
                    li[1, o:o + 8, :] = _pk2(ai, bi)
                    li[2, o:o + 8, :] = _pk2(ar, br)

    def i_op(ch):
        base = 0
        for dr, di in cdft(li, 128 * len(ch), True):
            do[0, base:base + dr.shape[0], :] = dr
            do[1, base:base + dr.shape[0], :] = di
            base += dr.shape[0]
            sync[0] = None

    def s3_job(ch, it):
        def gen():
            for gp, pair in enumerate(ch):
                for gi, g in enumerate(pair):
                    if g is None:
                        continue
                    t = []
                    for n0 in range(4):
                        a4 = []
                        for n1 in range(4):
                            k = 4 * n1 + n0
                            rws = dyn(gp * 256 + (k // 2) * 32 + 2 * (k % 2) + gi, 8, 0, 4)
                            a4.append(twid(k, do[0, rws, :], do[1, rws, :], +1))
                        t.append(_fft16_a(a4, n0, +1))
                        yield token(t[-1][1][0], t[-1][3][1], t[-1][0][0], t[-1][2][1])
                    for k0 in range(4):
                        o = _radix4([t[n0][k0] for n0 in range(4)], +1)
                        pks = []
                        for k1 in range(4):
                            n = k0 + 4 * k1
                            yr, yi = o[k1]
                            if g == 32:
                                nyb[n] = yr
                                pks.append(yr)
                                continue
                            if g == 0:
                                yi = jnp.where(row8 + it == 0, nyb[n, dyn(0, 8), :], yi)
                            pks.append(_pk2(yr, yi))
                            yp[n, pl.ds(blk(it, 32, 8 * g), 8), :] = pks[-1]
                        yield token(*pks)
        return Job(gen(), 8 * sum(ngr(p) for p in ch))

    def ny1_job():
        def gen():
            zero = jnp.zeros((8, 128), f32)
            t = []
            for n0 in range(4):
                t.append(_fft16_a([(x1[4 * n1 + n0, dyn(512, 8), :], zero) for n1 in range(4)], n0, -1))
                yield token(t[-1][1][0], t[-1][3][1], t[-1][0][0], t[-1][2][0])
            acc = [[zero, zero], [zero, zero]]
            for k0 in range(4):
                o = _radix4([t[n0][k0] for n0 in range(4)], -1)
                for k1 in range(4):
                    k = k0 + 4 * k1
                    v = twid(k, o[k1][0], o[k1][1], -1)
                    acc[k % 2] = [jnp.where(row8 == k // 2, v[e], acc[k % 2][e]) for e in range(2)]
                yield token(*acc[k0 % 2])
            (ar, ai), (br, bi) = acc
            tri = (_pk2(ar + ai, br + bi), _pk2(ai, bi), _pk2(ar, br))
            for n in range(3):
                lf[n, 0:8, :] = tri[n]
            yield token(*tri)
        return Job(gen(), 9)

    def ny_f():
        (xr, xi), = cdft(lf, 8, False)
        wr_ = _bf(wtr[0, dyn(256, 8), :]).astype(f32)
        wi_ = _bf(wti[0, dyn(256, 8), :]).astype(f32)
        yr, yi = xr * wr_ - xi * wi_, xr * wi_ + xi * wr_
        for n, v in enumerate((yr + yi, yi, yr)):
            li[n, 0:8, :] = _pk(v)

    def ny_i():
        (dr, di), = cdft(li, 8, True)
        do[0, 0:16, :] = dr
        do[1, 0:16, :] = di

    def ny3_job():
        def gen():
            t = []
            for n0 in range(4):
                a4 = []
                for n1 in range(4):
                    k = 4 * n1 + n0
                    r = 2 * (k % 8) + k // 8
                    re, im = (jnp.broadcast_to(do[e, pl.ds(zr[0] + r, 1), :], (8, 128)) for e in range(2))
                    a4.append(twid(k, re, im, +1))
                t.append(_fft16_a(a4, n0, +1))
                yield token(t[-1][1][0], t[-1][3][1], t[-1][0][0], t[-1][2][1])
            for k0 in range(4):
                o = _radix4([t[n0][k0] for n0 in range(4)], +1)
                for k1 in range(4):
                    nyb[k0 + 4 * k1] = o[k1][0]
                yield token(*[o[k1][0] for k1 in range(4)])
        return Job(gen(), 8)

    def si_tile(j, fused):
        e0 = _dot(_bf(yp[j, dyn(0, 64), :]), _bf(cb[328:392, 0:128]), _TN)
        e2 = _dot(_bf(yp[j, dyn(128, 64), :]), _bf(cb[328:392, 128:256]), _TN)
        y13 = jnp.concatenate([yp[j, dyn(64, 64), :], yp[j, dyn(192, 64), :]], axis=0)
        pq = _dot(_bf(y13), _bf(cb[200:328, :]), _TN)
        p, q = pq[:, 0:128], pq[:, 128:256]
        ep, em = e0 + e2, e0 - e2
        sync[0] = None
        st = jnp.concatenate([ep + p, em + q, ep - p, em - q], axis=1)
        rs = slice(j * 128, (j + 1) * 128)
        if fused:
            ob[rs, :] = (xb[rs, :].astype(f32) + st * gate[dyn(j * 128, 128), :]).astype(jnp.bfloat16)
        else:
            sbuf[j // 4] = st

    d0, d1 = dyn(0, MQ, 0), dyn(0, MQ, 1)

    def strassen(prod, bufs, out):
        put, get = bufs
        put(0, prod(0))
        yield
        m = prod(1)
        put(1, m)
        put(2, get(0, 0) - m)
        yield
        m = prod(2)
        put(3, m)
        put(4, get(2, 0) + m)
        yield
        out(1, 1, prod(3) + get(4, 0))
        yield
        m = prod(4)
        out(0, 1, get(3, 0) + m)
        put(5, get(0, 1) - m)
        yield
        m = prod(5)
        out(1, 0, get(1, 0) + m)
        put(6, get(5, 0) + m)
        yield
        out(0, 0, prod(6) + get(6, 0))
        yield

    def g_quad(q, jobs, after):
        cur = [0]
        vb_ = (va, vb, vc, vd, ve, vf, vg)
        ub_ = (ua, ub, uc, ud, ue, uf, ug)

        def prod(n, m):
            lhs = jnp.concatenate([sa[kt, 7 * n + m, dyn(0, MQ // 2), :] for kt in range(4)], axis=1)
            if n in _RDIR and m in _RDIR:
                kq, tn = 2 * _RDIR[n][0] + _RDIR[m][0], 2 * _RDIR[n][1] + _RDIR[m][1]
                w = wspb[pl.ds(blk(q, 128, tn * KQ), 128), kq * KQ:(kq + 1) * KQ]
            else:
                t, ix = tslot(n, m)
                w = _bf(t[ix, dyn(0, 64), :])
            tk = spread(jobs.get(cur[0], []), 22)
            r = _dot(_bf(synced(lhs)), w, _NT)
            sync[0] = token(r[MQ - SYL:MQ - SYL + 8])
            return tiev(r, tk)

        def vput(k, v):
            vb_[k][0:MQ, :] = v

        def vget(k, w):
            return vb_[k][d1 if w else d0, :]

        def emit(half, tile, m2, tn, c):
            tq = tn + 2 * tile
            j = q + 4 * tq
            lo = half * MH + m2 * MQ
            n = min(MQ, FH - lo)
            hv = gelu2(y1s[j, dyn(lo, n), :]) * (c[0:n] + bbc[j, dyn(0, 8), :][0:1])
            hbufs[tq][lo // 2:(lo + n) // 2, :] = _pk(hv)

        def combine(n, m2, tn, m):
            s = 2 * m2 + tn

            def put(k, v):
                ub_[k][s, 0:MQ, :] = v

            def get(k, w):
                return ub_[k][s, d1 if w else d0, :]

            if n == 0:
                put(0, m)
            elif n == 1:
                put(1, m)
                put(2, get(0, 0) - m)
            elif n == 2:
                put(3, m)
                put(4, get(2, 0) + m)
            elif n == 3:
                emit(1, 1, m2, tn, m + get(4, 0))
            elif n == 4:
                emit(0, 1, m2, tn, get(3, 0) + m)
                put(5, get(0, 1) - m)
            elif n == 5:
                emit(1, 0, m2, tn, get(1, 0) + m)
                put(6, get(5, 0) + m)
            else:
                emit(0, 0, m2, tn, m + get(6, 0))

        for n in range(7):
            for _ in strassen(lambda m, n=n: prod(n, m), (vput, vget),
                              lambda i, j, v, n=n: combine(n, i, j, v)):
                for fn in after.get(cur[0], []):
                    fn()
                cur[0] += 1

    def tjobs(jobs, q, last=False):
        over(jobs, tprep_job(q, 1), 0, 27)
        if not last:
            over(jobs, tprep_job(q + 1, 0), 29, 49)

    jobs, after = {}, {}
    Q0 = CFG["q0"]
    over(jobs, wout_job(), *Q0["wo"])
    over(jobs, wprep_a_job(), *Q0["wa"])
    over(jobs, wprep_b_job(), *Q0["wb"])
    tjobs(jobs, 0)
    over(jobs, ny1_job(), *Q0["s1"])
    add(after, Q0["f"], ny_f)
    add(after, Q0["i"], ny_i)
    over(jobs, ny3_job(), *Q0["s3"])
    add(after, 37, lambda: o_tile(0, 2, False))
    add(after, 41, lambda: o_tile(0, 3, False))
    g_quad(0, jobs, after)
    wait(grp_4)

    def p2_body(it, carry):
        sync[0] = None
        q = 1 + it
        jobs, after = {}, {}
        for c in range(4):
            ch = [(8 * c, 8 * c + 1), (8 * c + 2, 8 * c + 3)]
            a1, b1, a3, b3 = CFG["fs"][c]
            over(jobs, s1_job(ch, it), a1, b1 + 1)
            add(after, CFG["tf"][c], lambda ch=ch: f_op(ch, it))
            add(after, CFG["tf"][c] + 3, lambda ch=ch: i_op(ch))
            over(jobs, s3_job(ch, it), a3, b3 + 1)
        tjobs(jobs, q)
        add(after, 2, lambda: o_tile(q - 1, 0, False))
        add(after, 6, lambda: o_tile(q - 1, 1, False))
        add(after, 38, lambda: o_tile(q, 2, False))
        add(after, 43, lambda: o_tile(q, 3, False))
        g_quad(q, jobs, after)
        return carry

    jax.lax.fori_loop(0, 2, p2_body, 0)
    sync[0] = None

    outs = []

    def out_dma(lo, hi, bases=(0, 4, 8, 12)):
        for base in bases:
            outs.append(o_cp(base + lo, base + hi))
            outs[-1].start()

    jobs, after = {}, {}
    tjobs(jobs, 3, last=True)
    add(after, 2, lambda: o_tile(2, 0, False))
    add(after, 5, lambda: o_tile(2, 1, False))
    gated = [j for j in range(NB) if j % 4 != 3]
    for n in range(6):
        add(after, 7 + 3 * n, lambda n=n: (si_tile(gated[2 * n], True), si_tile(gated[2 * n + 1], True)))
    add(after, 26, lambda: (si_tile(3, False), si_tile(7, False)))
    add(after, 29, lambda: (si_tile(11, False), si_tile(15, False)))
    add(after, 31, lambda: out_dma(0, 3))
    add(after, 43, lambda: o_tile(3, 2, True))
    add(after, 48, lambda: o_tile(3, 3, True))
    g_quad(3, jobs, after)
    o_tile(3, 0, True)
    out_dma(3, 4, (8, 12))
    o_tile(3, 1, True)
    out_dma(3, 4, (0,))
    out_dma(3, 4, (4,))
    wait(outs)


@jax.jit
def pallas_recurrent_scan__spectral_gfnet__mixer_gmlp__prompt_kernel(
    A_x: jax.Array,
    A_w_r: jax.Array,
    A_w_i: jax.Array,
    B_x: jax.Array,
    B_w_in: jax.Array,
    B_w_sp: jax.Array,
    B_b_sp: jax.Array,
    B_w_out: jax.Array,
):
    del B_x
    bf16, f32, u32 = jnp.bfloat16, jnp.float32, jnp.uint32
    hbm_spec = pl.BlockSpec(memory_space=pltpu.HBM)
    scratch = [
        pltpu.VMEM((S, D), bf16),
        pltpu.VMEM((F, D), bf16),
        pltpu.VMEM((F // 2, D), u32),
        pltpu.VMEM((FH, D), bf16),
        pltpu.VMEM((FHP // 2, D), u32),
        pltpu.VMEM((S, S), bf16),
        pltpu.VMEM((4 * S,), bf16),
        pltpu.VMEM((NB, 32, 128), f32),
        pltpu.VMEM((257, S), bf16),
        pltpu.VMEM((257, S), bf16),
        pltpu.VMEM((2, S // 2, 128), u32),
        pltpu.VMEM((2, S // 2, 128), u32),
        pltpu.VMEM((S // 2, 128), u32),
        pltpu.VMEM((8, 264, 128), u32),
        pltpu.VMEM((8, 264, 128), u32),
        pltpu.VMEM((528, 256), u32),
        pltpu.VMEM(_TW.shape, f32),
        pltpu.VMEM((9, 64, 256), u32),
        pltpu.VMEM((9, 64, 256), u32),
        pltpu.VMEM((7, MH // 2, 256), u32),
    ] + [pltpu.VMEM((MH, 128), f32)] * 10 + [
    ] + [pltpu.VMEM((64, 768), u32)] * 4 + [
        pltpu.VMEM((2, 256, 128), f32),
        pltpu.VMEM((2, 256, 128), f32),
        pltpu.VMEM((32, 128), f32),
        pltpu.VMEM((32, 128), f32),
        pltpu.VMEM((NB, 544, 128), f32),
        pltpu.VMEM((NB, 2 * MH, 128), f32),
    ] + [pltpu.VMEM((2 * MH, 128), f32)] * 4 + [
        pltpu.VMEM((7, MH, 128), f32),
        pltpu.VMEM((7, MH, 128), f32),
        pltpu.VMEM((4, 49, 96, 128), u32),
        pltpu.VMEM((28, 64, KQ), u32),
        pltpu.VMEM((21, 64, KQ), u32),
    ] + [pltpu.VMEM((4, 192, 128), f32)] * 7 + [
    ] + [pltpu.VMEM((192, 128), f32)] * 7 + [
    ] + [pltpu.VMEM((MH, 128), u32)] * 4 + [
        pltpu.VMEM((3, 256, 128), u32),
        pltpu.VMEM((3, 256, 128), u32),
        pltpu.VMEM((2, 512, 128), f32),
        pltpu.VMEM((NB, 8, 128), f32),
        pltpu.VMEM((NB, 256, 128), u32),
        pltpu.VMEM((S, D), f32),
        pltpu.VMEM((4, 128, D), f32),
        pltpu.VMEM((S, D), bf16),
        pltpu.SMEM((8,), jnp.int32),
        pltpu.SemaphoreType.DMA((11,)),
    ]
    return pl.pallas_call(
        _kernel,
        in_specs=[hbm_spec] * 10,
        out_specs=hbm_spec,
        out_shape=jax.ShapeDtypeStruct(A_x.shape, A_x.dtype),
        scratch_shapes=scratch,
        compiler_params=pltpu.CompilerParams(vmem_limit_bytes=110 * 1024 * 1024),
    )(A_x, A_w_r.T, A_w_i.T, B_w_in.T, B_w_sp, B_b_sp, B_w_out, jnp.asarray(_CB), jnp.asarray(_TW),
      jnp.asarray(np.zeros((8,), np.int32)))
```

```python
import math

import jax
import jax.numpy as jnp
import numpy as np
import jax.experimental.pallas as pl
import jax.experimental.pallas.tpu as pltpu

S = 2048
D = 512
F = 1376
FH = 688
FHP = 768
NB = 16
NX = 528
EPS = 1e-5

_C = math.sqrt(2.0 / math.pi)
_A = 0.044715
KAPPA = (_C * _A) ** (1.0 / 3.0)
BETA = _C / KAPPA
EPS2 = 4.0 * KAPPA * KAPPA * EPS
INV4K = 1.0 / (4.0 * KAPPA)

_NT = (((1,), (1,)), ((), ()))
_NN = (((1,), (0,)), ((), ()))
_TN = (((0,), (0,)), ((), ()))


def _pack_rows(m):
    u = np.ascontiguousarray(m, dtype=np.float32).view(np.uint32).astype(np.uint64)
    b = ((u + 0x7FFF + ((u >> 16) & 1)) >> 16).astype(np.uint32)
    return b[0::2] | (b[1::2] << 16)


def _tables():
    n2 = np.arange(128)
    gf = np.zeros((4, 128, 256))
    mi = np.zeros((4, 128, 256))
    for c in range(4):
        for j in range(64):
            k = 4 * j + c
            th = 2 * np.pi * k * n2 / 512
            co, si = np.cos(th), np.sin(th)
            m, r = j // 8, j % 8
            re = 16 * m + r
            im = re + 8
            kre, kim = re, im
            w = 1.0 if k == 0 else 2.0
            if c in (0, 2):
                gf[c, re, :128], gf[c, im, :128] = co, -si
                mi[c, kre, :128], mi[c, kim, :128] = w * co, -w * si
            elif c == 1:
                gf[c, re, :128], gf[c, re, 128:] = co, -si
                gf[c, im, :128], gf[c, im, 128:] = -si, -co
                mi[c, kre, :128], mi[c, kim, :128] = w * co, -w * si
                mi[c, kre, 128:], mi[c, kim, 128:] = -w * si, -w * co
            else:
                gf[c, re, :128], gf[c, re, 128:] = co, si
                gf[c, im, :128], gf[c, im, 128:] = -si, co
                mi[c, kre, :128], mi[c, kim, :128] = w * co, -w * si
                mi[c, kre, 128:], mi[c, kim, 128:] = w * si, w * co
    nyq = np.cos(np.pi * n2)
    g0 = np.zeros((144, 128))
    g0[:128] = gf[0, :, :128]
    g0[128:136] = nyq
    g2 = np.zeros((144, 128))
    g2[:128] = gf[2, :, :128]
    mi[0, 8, :128] = nyq
    godd = np.zeros((256, 256))
    for n, c in enumerate((1, 3)):
        ks = 4 * np.arange(64) + c
        th = 2 * np.pi * np.outer(ks, n2) / 512
        godd[64 * n:64 * n + 64, :128] = np.cos(th) - np.sin(th)
        godd[64 * n:64 * n + 64, 128:] = (np.cos(th) + np.sin(th)) * (-1.0 if c == 1 else 1.0)
        godd[128:192, 128 * n:128 * n + 128] = np.cos(th)
    fs = 1.0 / KAPPA
    bs = 1.0 / (S * D)
    cc = np.cos(2 * np.pi * np.outer(n2, n2) / 128)
    ss = np.sin(2 * np.pi * np.outer(n2, n2) / 128)
    cb = np.concatenate(
        [
            godd * fs,
            np.concatenate([g0, g2], 1) * fs,
            mi[1] * bs,
            mi[3] * bs,
            np.concatenate([mi[0, :, :128], mi[2, :, :128]], 1) * bs,
            np.concatenate([cc, np.zeros((128, 128))], 1),
            np.concatenate([ss - cc, -ss - cc], 1),
        ],
        0,
    )
    k1 = np.arange(16)
    ph = 2 * np.pi * np.outer(k1, n2) / 2048
    tw = np.concatenate([np.cos(ph), np.sin(ph)], 1)
    tw = np.repeat(tw, 8, axis=0).astype(np.float32)
    return _pack_rows(cb), tw


_CB, _TW = _tables()


def _bf(u32):
    return pltpu.bitcast(u32, jnp.bfloat16)


def _u32(bf):
    return pltpu.bitcast(bf, jnp.uint32)


def _bits(f):
    return jax.lax.bitcast_convert_type(f, jnp.uint32)


def _dot(a, b, dims):
    return jax.lax.dot_general(a, b, dims, preferred_element_type=jnp.float32)


def _pk(v):
    return _u32(v.astype(jnp.bfloat16))


def _pk2(a, b):
    return _pk(jnp.concatenate([a, b], axis=0))


def _unpk(u):
    lo = jax.lax.bitcast_convert_type(u << 16, jnp.float32)
    hi = jax.lax.bitcast_convert_type(u & jnp.uint32(0xFFFF0000), jnp.float32)
    return lo, hi


def _radix4(a, sign):
    (ar, ai), (br, bi), (cr, ci), (dr, di) = a
    s0r, s0i = ar + cr, ai + ci
    d0r, d0i = ar - cr, ai - ci
    s1r, s1i = br + dr, bi + di
    d1r, d1i = br - dr, bi - di
    o0 = (s0r + s1r, s0i + s1i)
    o2 = (s0r - s1r, s0i - s1i)
    if sign < 0:
        o1 = (d0r + d1i, d0i - d1r)
        o3 = (d0r - d1i, d0i + d1r)
    else:
        o1 = (d0r - d1i, d0i + d1r)
        o3 = (d0r + d1i, d0i - d1r)
    return [o0, o1, o2, o3]


def _tw16(x, e, sign):
    e = e % 16
    xr, xi = x
    if e == 0:
        return x
    if e == 4:
        return (xi, -xr) if sign < 0 else (-xi, xr)
    if e in (2, 6):
        h = math.sqrt(0.5)
        if e == 2:
            if sign < 0:
                return ((xr + xi) * h, (xi - xr) * h)
            return ((xr - xi) * h, (xi + xr) * h)
        if sign < 0:
            return ((xi - xr) * h, (xr + xi) * (-h))
        return ((xr + xi) * (-h), (xr - xi) * h)
    ang = sign * 2 * math.pi * e / 16
    wr, wi = math.cos(ang), math.sin(ang)
    return (xr * wr - xi * wi, xr * wi + xi * wr)


def _fft16_a(a4, n0, sign):
    o = _radix4(a4, sign)
    return [_tw16(o[k0], n0 * k0, sign) for k0 in range(4)]


MH = 352
MQ = 176
KQ = S // 4
SYL = 144

CFG = dict(
    q0=dict(wo=[1, 7], wa=[8, 21], wb=[22, 48], s1=[8, 20], f=28, i=31, s3=[34, 44]),
    tf=[5, 14, 23, 32], fs=[[0, 4, 10, 13], [6, 9, 19, 22], [15, 18, 28, 36], [24, 27, 39, 48]],
    lsn=0, l2r=[0, 7], lnw=24, lnb=8, win=5, l1e=True, tz2=[0, 0, 8, 16], tz1=[6, 6, 6, 6, 0, 0, 0],
)


def _str_l(a11, a12, a21, a22):
    if a22 is None:
        return (a11, a21, a11, -a11 if a21 is None else a21 - a11, a11 + a12, None, a12)
    return (a11 + a22, a21 + a22, a11, a21 - a11, a11 + a12, a22, a12 - a22)


def _str_r(b11, b21, b12, b22):
    return (b11 + b22, b11, b12 - b22, b11 + b12, b22, b21 - b11, b21 + b22)


_SUMS_L, _SUMS_R = (0, 1, 3, 4, 6), (0, 2, 3, 5, 6)
_RDIR = {1: (0, 0), 4: (1, 1)}


def _kernel(
    x_hbm, wr_hbm, wi_hbm, win_hbm, wsp_hbm, b_hbm, wout_hbm, cb_hbm, tw_hbm, z_hbm,
    o_hbm,
    xb, winb, wint, woutb, woutp, wspb, bb, bbc, wrb, wib, w32r, w32i, w32n, wtr, wti,
    cb, tw, xs0, xs1, wz, qa, qb, qc, qd, qe, qf, qg, qh, qi, qj, ys0, ys1, ys2, ys3, ls0, ls1, st_m, st_r,
    x1, y1s, zf0, zf1, zf2, zf3, xa0, sa, tbx, tby, ua, ub, uc, ud, ue, uf, ug, va, vb, vc, vd, ve, vf, vg,
    hlo, hhi, lf, li, do, nyb, yp, gate, sbuf, ob, zs, sems,
):
    f32, u32 = jnp.float32, jnp.uint32
    nsem = [0]

    def cp(src, dst):
        return pltpu.make_async_copy(src, dst, sems.at[nsem[0]])

    def group(*cps):
        nsem[0] += 1
        return [c for x in cps for c in (x if isinstance(x, list) else [x])]

    def rows(ref, lo, hi):
        return ref.at[pl.ds(lo, hi - lo), :]

    def xcp(lo, hi):
        return cp(x_hbm.at[0, pl.ds(lo * 128, (hi - lo) * 128), :], rows(xb, lo * 128, hi * 128))

    def wspcp(lo, hi):
        return [cp(rows(wsp_hbm, h + lo, h + hi), rows(wspb, h + lo, h + hi)) for h in (0, KQ, 2 * KQ, 3 * KQ)]

    def o_cp(lo, hi):
        return cp(rows(ob, lo * 128, hi * 128), o_hbm.at[0, pl.ds(lo * 128, (hi - lo) * 128), :])

    grp_z = group(cp(z_hbm, zs))
    grp_a = group(xcp(0, 1))
    grp_b = group(xcp(8, 9), cp(rows(win_hbm, FH, FH + MH), rows(winb, FH, FH + MH)))
    grp_c = group(cp(rows(win_hbm, FH + MH, F), rows(winb, FH + MH, F)), xcp(4, 5), xcp(12, 13))
    grp_d = group(cp(rows(win_hbm, 0, FH), rows(winb, 0, FH)), cp(rows(cb_hbm, 0, 200), rows(cb, 0, 200)),
                  xcp(1, 2), xcp(9, 10))
    grp_1 = group(xcp(5, 6), xcp(13, 14), xcp(2, 3), xcp(10, 11), wspcp(0, 48))
    grp_2 = group(xcp(6, 8), xcp(14, 16), xcp(3, 4), xcp(11, 12), wspcp(48, 128))
    grp_3 = group(wspcp(128, 256), cp(wr_hbm, wrb), cp(wi_hbm, wib), cp(wout_hbm, woutb),
                  cp(rows(cb_hbm, 200, 520), rows(cb, 200, 520)), cp(tw_hbm, tw))
    grp_3 += group(cp(b_hbm, bb.at[pl.ds(0, S)]))
    grp_4 = group(wspcp(256, 512))

    def wait(grp):
        for c_ in grp:
            c_.wait()

    for c_ in grp_z + grp_a + grp_b + grp_c + grp_d + grp_1 + grp_2 + grp_3 + grp_4:
        c_.start()
    wait(grp_z + grp_a)

    zr = [zs[n] for n in range(3)]
    zvec = jnp.full((8, 128), zr[2], jnp.int32).astype(u32)

    def dyn(lo, n, w=0, stride=None):
        if stride is None:
            return pl.ds(pl.multiple_of(zr[w] + lo, 8), n)
        return pl.ds(zr[w] + lo, n, stride=stride)

    def blk(i, n, extra=0):
        if isinstance(i, int):
            return i * n + extra
        return pl.multiple_of(i * n + extra, 8)

    def token(*vs):
        acc = None
        for v in vs:
            if v.dtype != u32:
                v = _bits(v)
            for r in range(0, v.shape[0], 8):
                for c in range(0, v.shape[1], 128):
                    t = v[r:r + 8, c:c + 128]
                    acc = t if acc is None else acc | t
        return acc

    sync = [None]

    def synced(u):
        if sync[0] is None:
            return u
        sz = sync[0] & zvec
        cols = [u[0:8, c:c + 128] | sz for c in range(0, u.shape[1], 128)]
        return jnp.concatenate([jnp.concatenate(cols, axis=1), u[8:]], axis=0)

    def tiev(v, toks):
        parts = []
        prev = 0
        for r in sorted(toks):
            if r * 8 > prev:
                parts.append(v[prev:r * 8])
            parts.append(jax.lax.bitcast_convert_type(_bits(v[r * 8:r * 8 + 8]) | (toks[r] & zvec), f32))
            prev = r * 8 + 8
        if prev < v.shape[0]:
            parts.append(v[prev:])
        return jnp.concatenate(parts, axis=0) if len(parts) > 1 else parts[0]

    ALL = 9999
    rel = [None]

    def gate_(v):
        if rel[0] is None:
            return v
        u = v if v.dtype == u32 else _bits(v)
        tiles = [[u[r:r + 8, c:c + 128] | rel[0] for c in range(0, u.shape[1], 128)]
                 for r in range(0, u.shape[0], 8)]
        u = jnp.concatenate([jnp.concatenate(t, axis=1) for t in tiles], axis=0)
        return u if v.dtype == u32 else jax.lax.bitcast_convert_type(u, v.dtype)

    class Job:
        def __init__(self, gen, n, win=None):
            self.gen, self.left, self.win = gen, n, CFG["win"] if win is None else win

        def __next__(self):
            self.left -= 1
            return next(self.gen)

    def spread(lists, nslot, src=None):
        out = {}
        rels = {}
        for job, n, lo, hi in lists:
            n = min(n, job.left)
            for k in range(n):
                sl = min(int(nslot * (lo + (k + 0.5) * (hi - lo) / n)), nslot - 1)
                rs = sl - job.win
                if src is not None and rs >= 0:
                    if rs not in rels:
                        rels[rs] = _bits(src[8 * rs:8 * rs + 8]) & zvec
                    rel[0] = rels[rs]
                tk = next(job)
                rel[0] = None
                out[sl] = tk if sl not in out else out[sl] | tk
        return out

    def add(d, k, v):
        d.setdefault(k, []).append(v)

    def over(jobs, job, lo, hi):
        n = -(-job.left // (hi - lo))
        for pos in range(lo, hi):
            add(jobs, pos, (job, n if pos < hi - 1 else ALL, 0.0, 1.0))

    xsb, ysb, zfb = (xs0, xs1), (ys0, ys1, ys2, ys3), (zf0, zf1, zf2, zf3)
    TOFF = (0, 8, 4, 12)
    row8 = jax.lax.broadcasted_iota(jnp.int32, (8, 128), 0)

    def ln_stats(x):
        m = jnp.sum(x, axis=-1, keepdims=True) * (1.0 / D)
        v = jnp.sum(x * x, axis=-1, keepdims=True) * (1.0 / D) - m * m
        return m, jax.lax.rsqrt(jnp.maximum(v, 0.0) + EPS) * KAPPA

    def xrows(i, r):
        return xb[pl.ds(blk(i, 128, r), 16), :].astype(f32)

    def lns_job(i, p):
        def gen():
            for r in range(0, 128, 16):
                for e in range(2):
                    x = gate_(xrows(i + 8 * e, r))
                    sts = [ln_stats(x[8 * hf:8 * hf + 8]) for hf in range(2)]
                    st = [jnp.broadcast_to(sts[hf][n], (8, 128)) for n in range(2) for hf in range(2)]
                    for n, v in enumerate(st):
                        (ls1 if p else ls0)[e, 2 * r + 8 * n:2 * r + 8 * n + 8, :] = v
                    yield token(*st)
        return Job(gen(), 16, CFG["lnw"])

    def ln_rows(i, b, r, pre=False):
        if pre:
            x = xrows(i, r)
            ls = ls1 if b // 2 else ls0
            m, rs = gate_(ls[b % 2, dyn(2 * r, 16), :]), ls[b % 2, dyn(2 * r + 16, 16), :]
            a0, a1, a2, a3 = ((x[:, 128 * j:128 * (j + 1)] - m) * rs for j in range(4))
            xn = jnp.concatenate([a0, a1, a2, a3], axis=1)
        else:
            x = gate_(xrows(i, r))
            m, rs = ln_stats(x)
            xn = (x - m) * rs
            a0, a1, a2, a3 = (xn[:, 128 * j:128 * (j + 1)] for j in range(4))
        s02, s13 = a0 + a2, a1 + a3
        p, q = a0 - a2, a1 - a3
        ys = [s02 + s13, s02 - s13, p, q, p + q, p - q]
        ysb[b][r // 2:r // 2 + 8, :] = _pk(jnp.concatenate(ys, axis=1))
        for hf in range(2):
            xsb[b // 2].at[PLAIN[b % 2][hf]][r // 2:r // 2 + 8, :] = _pk(xn[:, 256 * hf:256 * (hf + 1)])
        return xn, token(ys[0], ys[1], ys[4], ys[5])

    PLAIN = ((1, 7), (8, 4))

    def ln_job(i, b):
        def gen():
            for r in range(0, 128, 16):
                yield ln_rows(i, b, r)[1]
        return Job(gen(), 8, CFG["lnw"])

    def lnp_job(i, p, win=None, pre=True):
        def gen():
            for r in range(0, 128, 16):
                a, tk = ln_rows(i, 2 * p, r, pre)
                yield tk
                b, tk = ln_rows(i + 8, 2 * p + 1, r, pre)
                ops = _str_r(a[:, 0:256], a[:, 256:512], b[:, 0:256], b[:, 256:512])
                for n in _SUMS_R:
                    xsb[p].at[n][r // 2:r // 2 + 8, :] = _pk(ops[n])
                yield token(tk, *[ops[n] for n in _SUMS_R])
        return Job(gen(), 16, CFG["lnw"] if win is None else win)

    def wz_job():
        def ld(r, lanes):
            return gate_(winb[r:r + 16, lanes].astype(f32))

        def gen():
            for r in range(0, MH, 16):
                for c in range(2):
                    lo, hi = slice(c * 128, (c + 1) * 128), slice(256 + c * 128, 256 + (c + 1) * 128)
                    a11, a12 = ld(r, lo), ld(r, hi)
                    bot = (ld(MH + r, lo), ld(MH + r, hi)) if MH + r < FH else (None, None)
                    ops = _str_l(a11, a12, *bot)
                    for n in range(7):
                        if ops[n] is None:
                            wz.at[n][r // 2:r // 2 + 8, lo] = jnp.zeros((8, 128), u32)
                        else:
                            wz.at[n][r // 2:r // 2 + 8, lo] = _pk(ops[n])
                    yield token(*[ops[n] for n in _SUMS_L if ops[n] is not None])
        return Job(gen(), 44)

    def gelu2(z):
        return z + z * jnp.tanh(z * (z * z + BETA))

    def cdot(r0, r1, lanes, w):
        outs = []
        r = r0
        while r < r1:
            n = min(64, r1 - r)
            if r1 - r - n == 16:
                n += 16
            outs.append(_dot(_bf(cb[r // 2:(r + n) // 2, lanes]), w, _NT))
            r += n
        return jnp.concatenate(outs, axis=0)

    L0, L1 = slice(0, 128), slice(128, 256)

    def l1_job(kq):
        xa = xa0
        G = 32

        def nrm(e, lo, n, mg):
            z = zfb[2 * kq + e][dyn(lo, n, 1), :].reshape(n // 8, 8, 128)
            return ((z - mg[e]) * st_r[dyn(8 * (2 * kq + e), 8), :]).reshape(n, 128)

        def gen():
            for r in range(0, MH, G):
                n2 = min(G, FH - MH - r)
                mg = [gate_(st_m[dyn(8 * (2 * kq + e), 8), :]) for e in range(2)]
                top = [nrm(e, r, G, mg) for e in range(2)]
                bot = [nrm(e, MH + r, n2, mg) for e in range(2)]
                if n2 < G:
                    pad = jnp.zeros((G - n2, 128), f32)
                    bot = [jnp.concatenate([v, pad], axis=0) for v in bot]
                ops = _str_l(top[0], top[1], bot[0], bot[1])
                for n, v in enumerate(ops):
                    xa[n, r:r + G, :] = v
                yield token(*[ops[n] for n in _SUMS_L])
        return Job(gen(), 11)

    def l2_job(kt):
        def gen():
            for r in range(0, MQ, 16):
                zn = {}
                for e in range(2):
                    m, rs = gate_(st_m[dyn(8 * (2 + e), 8), :]), st_r[dyn(8 * (2 + e), 8), :]
                    for qd_ in range(4):
                        lo = qd_ * MQ + r
                        if lo < FH:
                            z = zfb[2 + e][dyn(lo, 16, 1), :].reshape(2, 8, 128)
                            zn[e, qd_] = ((z - m) * rs).reshape(16, 128)
                        else:
                            zn[e, qd_] = None
                l1 = [_str_l(zn[0, m2], zn[1, m2], zn[0, 2 + m2], zn[1, 2 + m2]) for m2 in range(2)]
                for n in range(7):
                    ops = _str_l(gate_(xa0[n, dyn(r, 16), :]), l1[0][n], xa0[n, dyn(MQ + r, 16), :], l1[1][n])
                    for m, v in enumerate(ops):
                        o = 7 * n + m
                        sa.at[kt, o // 2][r // 2:r // 2 + 8, (o % 2) * 128:(o % 2 + 1) * 128] = (
                            jnp.zeros((8, 128), u32) if v is None else _pk(v))
                    yield token(*[ops[m] for m in _SUMS_L])
        return Job(gen(), 77)

    def wprep_a_job():
        def gen():
            for b in range(NB):
                lanes = slice(b * 128, (b + 1) * 128)
                rws = slice(64 * b, 64 * (b + 1))
                for src, w32 in ((wrb, w32r), (wib, w32i)):
                    for j in range(2):
                        v = _u32(src[j * 128:(j + 1) * 128, lanes].T)
                        w32[j, rws, :] = v
                        yield token(v)
                nr, ni = (jnp.broadcast_to(src[256:257, lanes].astype(f32), (8, 128)) for src in (wrb, wib))
                slab = [jnp.where(row8 == 0, v, 0.0) for v in (nr, ni)] + [jnp.zeros((112, 128), f32)]
                v = _u32(jnp.concatenate(slab, axis=0).astype(jnp.bfloat16).T)
                w32n[rws, :] = v
                yield token(v)
        return Job(gen(), 80)

    def wprep_b_job():
        def gen():
            for r0 in range(8):
                tt = w32n[dyn(r0, 128, 0, 8), :].T[0:16]
                wtr[0, 256 + r0:257 + r0, :] = tt[0:1]
                wti[0, 256 + r0:257 + r0, :] = tt[8:9]
                yield token(tt)
            for r0 in range(8):
                for w32, wt in ((w32r, wtr), (w32i, wti)):
                    for j in range(2):
                        tt = w32[j, dyn(r0, 128, 0, 8), :].T
                        wt[r0, j * 128:(j + 1) * 128, :] = tt
                        yield token(tt)
        return Job(gen(), 40)

    def wout_job():
        def gen():
            woutp[FH // 2:FHP // 2, :] = jnp.zeros(((FHP - FH) // 2, D), u32)
            bvec = (bb[0:S].astype(f32) * INV4K).reshape(1, S)
            for j in range(NB):
                bbc[j, 0:8, :] = jnp.broadcast_to(bvec[:, j * 128:(j + 1) * 128], (8, 128))
            for c in range(4):
                lanes = slice(c * 128, (c + 1) * 128)
                for lo in range(0, FH, 64):
                    hi = min(lo + 64, FH)
                    v = _u32(woutb[lo:hi, lanes])
                    woutp[lo // 2:hi // 2, lanes] = v
                    yield token(v)
        return Job(gen(), 44)

    def tslot(n, m):
        return (tbx, 7 * n + m) if n < 4 else (tby, 7 * (n - 4) + m)

    def tprep_job(q, part, r_lo=0, nr=8):
        def gen():
            for rr in range(nr):
                r = r_lo + rr
                if not isinstance(r, int):
                    r = jnp.minimum(r, 7)
                ro = pl.ds(blk(r, 8), 8)
                for c in range(4):
                    lanes = slice(c * 128, (c + 1) * 128)

                    def up(tn, kq):
                        base = blk(q, 128, tn * KQ) + blk(r, 16)
                        if not isinstance(base, int):
                            base = pl.multiple_of(base, 16)
                        return gate_(wspb[pl.ds(base, 16), kq * KQ + c * 128:kq * KQ + (c + 1) * 128].astype(f32))

                    def level2(n, y):
                        ops = _str_r(y[0, 0], y[1, 0], y[0, 1], y[1, 1])
                        for m in range(7):
                            if n in _RDIR and m in _RDIR:
                                continue
                            t, ix = tslot(n, m)
                            t.at[ix][ro, lanes] = _pk(ops[m])
                        return token(*[ops[m] for m in _SUMS_R])

                    def cmb(a, b, sg):
                        return {k: a[k] + b[k] if sg > 0 else a[k] - b[k] for k in a}

                    def blk4(tn0, kq0):
                        return {(kq, tn): up(tn0 + tn, kq0 + kq) for kq in range(2) for tn in range(2)}

                    if part == 0:
                        b11 = blk4(0, 0)
                        yield level2(1, b11)
                        b22 = blk4(2, 2)
                        yield level2(0, cmb(b11, b22, 1))
                        b12 = blk4(2, 0)
                        yield level2(2, cmb(b12, b22, -1))
                        yield level2(3, cmb(b11, b12, 1))
                    else:
                        b22 = blk4(2, 2)
                        yield level2(4, b22)
                        b21 = blk4(0, 2)
                        yield level2(6, cmb(b21, b22, 1))
                        yield level2(5, cmb(b21, blk4(0, 0), -1))
        return Job(gen(), nr * 4 * (4 - part))

    def xplain(b, w):
        return _bf(jnp.concatenate([xsb[b // 2][n, dyn(0, 64, w), :] for n in PLAIN[b % 2]], axis=1))

    def z2_sink(b, lo, z, tk, st):
        CH = 4
        ng = z.shape[0] // 8
        marks = []
        for r in range(0, ng, CH):
            n = min(CH, ng - r)
            tkc = {k - r: v for k, v in tk.items() if r <= k < r + n}
            if len(marks) >= 2:
                tkc[0] = marks[-2] if 0 not in tkc else tkc[0] | marks[-2]
            y = gelu2(tiev(z[8 * r:8 * (r + n)], tkc))
            zfb[b][lo + 8 * r:lo + 8 * (r + n), :] = y
            for q in range(n):
                if "c" not in st:
                    st["c"] = y[0:8]
                    continue
                d = y[8 * q:8 * q + 8] - st["c"]
                st["sm"] = d if "sm" not in st else st["sm"] + d
                st["sq"] = d * d if "sq" not in st else st["sq"] + d * d
            marks.append(token(st["sm"], st["sq"]))
        st["n"] = st.get("n", 0) + ng
        if st["n"] == FH // 8:
            c, sm, sq, cnt = st["c"], st["sm"], st["sq"], FH // 8
            m2 = jnp.sum(sm + cnt * c, axis=0, keepdims=True) * (1.0 / FH)
            e = m2 - c
            v2 = jnp.sum(sq - 2.0 * e * sm + cnt * (e * e), axis=0, keepdims=True) * (1.0 / FH)
            st_m[8 * b:8 * b + 8, :] = jnp.broadcast_to(m2, (8, 128))
            st_r[8 * b:8 * b + 8, :] = jnp.broadcast_to(
                jax.lax.rsqrt(jnp.maximum(v2, 0.0) + EPS2) * INV4K, (8, 128))

    def z2_op(b, la, gated=True):
        z = _dot(_bf(wint[dyn(0, FH // 2), :]), xplain(b, 0), _NT)
        z2_sink(b, 0, z, spread(la, 86, z if gated else None), {})

    dq0, dq1 = dyn(0, MH, 0), dyn(0, MH, 1)

    def z1_chains(kt, jobs):
        rnd = [0]
        tks = []

        def pr(p, n):
            return _dot(_bf(synced(wz[n, dyn(0, MH // 2), :])), _bf(xsb[p][n, dyn(0, 64, 1), :]), _NT)

        def two(a, b):
            ra, rb = pr(*a), pr(*b)
            tks[:] = [spread(jobs.get(rnd[0], []), 42, ra)]
            sync[0] = token(ra[MH - SYL:MH - SYL + 8], rb[MH - SYL:MH - SYL + 8])
            rnd[0] += 1
            return ra, rb

        def tie1(v):
            return tiev(v, tks.pop()) if tks else v

        def out(b, lo, v):
            v = v[0:min(MH, FH - lo)]
            y1s[kt + TOFF[b], lo:lo + v.shape[0], :] = tie1(v)

        m1, m2 = two((0, 0), (0, 1))
        qa[...] = tie1(m1)
        qb[...] = m2
        qc[...] = m1 - m2
        m3, m6 = two((0, 2), (0, 3))
        out(1, MH, qc[dq0, :] + m3 + m6)
        qd[...] = m3
        m5, m4 = two((0, 4), (0, 5))
        out(1, 0, qd[dq0, :] + m5)
        out(0, MH, qb[dq0, :] + m4)
        qe[...] = qa[dq0, :] + m4 - m5
        m7, m1 = two((0, 6), (1, 0))
        out(0, 0, qe[dq0, :] + m7)
        qf[...] = m1
        m2, m3 = two((1, 1), (1, 2))
        qg[...] = tie1(m2)
        qh[...] = m3
        qi[...] = qf[dq0, :] - m2 + m3
        m6, m5 = two((1, 3), (1, 4))
        out(3, MH, qi[dq0, :] + m6)
        out(3, 0, qh[dq0, :] + m5)
        qj[...] = qf[dq1, :] - m5
        m4, m7 = two((1, 5), (1, 6))
        out(2, MH, qg[dq0, :] + m4)
        out(2, 0, qj[dq0, :] + m4 + m7)

    def d_op(i, b):
        y0, y2, p, q, pp, pm = (_bf(ysb[b][dyn(0, 64), 128 * n:128 * (n + 1)]) for n in range(6))
        o0 = cdot(256, 400, L0, y0)
        x1[i, 0:128, :] = o0[0:128]
        x1[i, 512:520, :] = o0[128:136]
        x1[i, 256:384, :] = cdot(256, 384, L1, y2)
        for n, (base, w) in enumerate(((128, pp), (384, pm))):
            t = cdot(128, 192, (L0, L1)[n], w)
            re = t + cdot(64 * n, 64 * n + 64, L1, q)
            im = cdot(64 * n, 64 * n + 64, L0, p) - t
            for m in range(8):
                x1[i, base + 16 * m:base + 16 * m + 8, :] = re[8 * m:8 * m + 8]
                x1[i, base + 16 * m + 8:base + 16 * m + 16, :] = im[8 * m:8 * m + 8]

    def p1_start():
        sts = [{}, {}]

        def z2_part(b, lo, hi, la):
            if b == 0:
                cols = []
                for c in range(4):
                    lanes = slice(c * 128, (c + 1) * 128)
                    cols.append(_u32(winb[FH + lo:FH + hi, lanes]))
                    wint[lo // 2:hi // 2, lanes] = cols[-1]
                lhs = jnp.concatenate(cols, axis=1)
            else:
                lhs = wint[dyn(lo // 2, (hi - lo) // 2), :]
            z = _dot(_bf(lhs), xplain(b, lo // MH), _NT)
            z2_sink(b, lo, z, spread(la, (hi - lo) // 8), sts[b])

        def z1_op(b, lb):
            if b == 0:
                cols = []
                for c in range(4):
                    lanes = slice(c * 128, (c + 1) * 128)
                    cols.append(_u32(winb[0:FH, lanes]))
                    wint[FH // 2:FH, lanes] = cols[-1]
                lhs = jnp.concatenate(cols, axis=1)
            else:
                lhs = wint[dyn(FH // 2, FH // 2), :]
            z = _dot(_bf(lhs), xplain(b, 1), _NT)
            y1s[TOFF[b], 0:FH, :] = tiev(z, spread(lb, 86, z))
            d_op(TOFF[b], b)

        lnj = ln_job(0, 0)
        while lnj.left:
            next(lnj)
        wait(grp_b)
        z2_part(0, 0, MH, [(ln_job(8, 1), ALL, 0.0, 0.6)])
        z2_part(1, 0, MH, [])
        wait(grp_c)
        ln4 = ln_job(4, 2)
        z2_part(0, MH, FH, [(ln4, 5, 0.0, 1.0)])
        z2_part(1, MH, FH, [(ln4, ALL, 0.0, 0.5)])
        z2_op(2, [(ln_job(12, 3), ALL, 0.0, 0.7)])
        z2_op(3, [(l1_job(0), ALL, 0.2, 1.0)])
        wait(grp_d)
        wzj, l2j, lnj = wz_job(), l2_job(0), lnp_job(1, 0, None, False)
        z1_op(0, [(l2j, 25, 0.0, 1.0), (wzj, 22, 0.0, 1.0)])
        z1_op(1, [(l2j, 25, 0.0, 1.0), (wzj, ALL, 0.0, 1.0)])
        z1_op(2, [(lnj, 8, 0.0, 1.0), (l2j, 14, 0.0, 1.0)])
        z1_op(3, [(lnj, ALL, 0.0, 0.8), (l2j, ALL, 0.0, 1.0)])

    def p1_quad(kt, bg):
        nk = jnp.minimum(kt + 1, 3)
        tz = CFG["tz2"]
        lnj = lnp_job(kt + 4, 1, CFG["lnb"])
        lsn = lns_job(nk, 0)
        z2_op(0, [(lns_job(kt + 4, 1), ALL, 0.0, 0.6), (lnj, 3, 0.75, 1.0), (bg, tz[0], 0.0, 1.0)])
        z2_op(1, [(lnj, ALL, 0.0, 0.8), (bg, tz[1], 0.0, 1.0)])
        z2_op(2, [(bg, tz[2], 0.0, 1.0), (l1_job(0), ALL, 0.2, 1.0)])
        z2_op(3, [(bg, tz[3], 0.0, 1.0), (lsn, CFG["lsn"], 0.0, 1.0)])
        d_op(kt, 0)
        d_op(kt + 8, 1)
        jobs = {}
        over(jobs, l2_job(kt), *CFG["l2r"])
        if lsn.left:
            over(jobs, lsn, 0, 4)
        over(jobs, lnp_job(nk, 0, CFG["lnb"]), 4, 7)
        for rn, n in enumerate(CFG["tz1"]):
            add(jobs, rn, (bg, n, 0.0, 1.0))
        z1_chains(kt, jobs)
        assert bg.left == 0
        d_op(kt + 4, 2)
        d_op(kt + 12, 3)

    p1_start()
    wait(grp_1)

    def p1_body(it, carry):
        @pl.when(it == 1)
        def _():
            wait(grp_2)

        sync[0] = None
        p1_quad(1 + it, tprep_job(0, 0, 3 * it, 3))
        return carry

    jax.lax.fori_loop(0, 3, p1_body, 0)
    sync[0] = None
    wait(grp_3)

    def hlanes(tn):
        return (hhi if tn // 2 else hlo), slice((tn % 2) * 128, (tn % 2 + 1) * 128)

    def o_tile(q, tn, fused):
        rs = pl.ds(blk(q, 128, tn * KQ), 128)
        h, hl = hlanes(tn)
        hp = jnp.concatenate([h[dyn(0, FH // 2), hl], jnp.zeros(((FHP - FH) // 2, 128), u32)], axis=0)
        w = _dot(_bf(hp), _bf(woutp[dyn(0, FHP // 2), :]), _TN)
        g = w + w * jnp.tanh(w)
        sync[0] = None
        if fused:
            ob[rs, :] = (xb[rs, :].astype(f32) + sbuf[tn, dyn(0, 128), :] * g).astype(jnp.bfloat16)
        else:
            gate[rs, :] = g

    def twid(k, re, im, sign):
        if k == 0:
            return re, im
        c = tw[8 * k:8 * k + 8, 0:128]
        s = tw[8 * k:8 * k + 8, 128:256]
        if sign < 0:
            return re * c + im * s, im * c - re * s
        return re * c - im * s, im * c + re * s

    def put3(dst, r0, a, b):
        sa_, sb_ = a[0] + a[1], b[0] + b[1]
        for n, (u, v) in enumerate(((sa_, sb_), (a[1], b[1]), (a[0], b[0]))):
            dst[r0:r0 + 8, 128 * n:128 * (n + 1)] = _pk2(u, v)
        return token(sa_, sb_)

    def s1_job(c, it):
        def gen():
            for gi in range(4):
                g = 8 * c + gi
                t = []
                for n0 in range(4):
                    a4 = [(x1[4 * n1 + n0, dyn(64 * it + 16 * g, 8), :],
                           x1[4 * n1 + n0, dyn(64 * it + 16 * g + 8, 8), :]) for n1 in range(4)]
                    t.append(_fft16_a(a4, n0, -1))
                    yield token(t[-1][1][0], t[-1][3][1], t[-1][0][0], t[-1][2][1])
                for kp in range(2):
                    oa = _radix4([t[n0][2 * kp] for n0 in range(4)], -1)
                    ob_ = _radix4([t[n0][2 * kp + 1] for n0 in range(4)], -1)
                    for k1 in range(4):
                        k = 4 * k1 + 2 * kp
                        yield put3(lf, 64 * gi + 4 * k, twid(k, *oa[k1], -1), twid(k + 1, *ob_[k1], -1))
        return Job(gen(), 48)

    def cdft(src, nrow, swap):
        m1 = _bf(cb[392:456, 0:128])
        m2 = _bf(cb[456:520, 0:128])
        m3 = _bf(cb[456:520, 128:256])
        if swap:
            m2, m3 = m3, m2
        n = max(nrow // 4, 8)
        for r in range(0, nrow, n):
            t1 = _dot(_bf(src[dyn(r, n), 0:128]), m1, _NN)
            yield (t1 + _dot(_bf(src[dyn(r, n), 128:256]), m2, _NN),
                   t1 + _dot(_bf(src[dyn(r, n), 256:384]), m3, _NN))
        sync[0] = None

    def cmul(xr, xi, wr_, wi_):
        return xr * wr_ - xi * wi_, xr * wi_ + xi * wr_

    def f_op(c, it):
        for gi, (xr, xi) in enumerate(cdft(lf, 256, False)):
            rws = dyn(32 * gi + c + 128 * it, 8, 0, 4)
            for pr in range(8):
                wr_, wi_ = _unpk(wtr[pr, rws, :]), _unpk(wti[pr, rws, :])
                ys = [cmul(xr[16 * pr + 8 * e:16 * pr + 8 * e + 8], xi[16 * pr + 8 * e:16 * pr + 8 * e + 8],
                           wr_[e], wi_[e]) for e in range(2)]
                put3(li, 64 * gi + 8 * pr, *ys)

    def i_op():
        for gi, (dr, di) in enumerate(cdft(li, 256, True)):
            do[0, 128 * gi:128 * (gi + 1), :] = dr
            do[1, 128 * gi:128 * (gi + 1), :] = di

    def s3_job(c, it):
        def gen():
            for gi in range(4):
                g = 8 * c + gi
                t = []
                for n0 in range(4):
                    a4 = []
                    for n1 in range(4):
                        k = 4 * n1 + n0
                        rws = dyn(128 * gi + 8 * k, 8)
                        a4.append(twid(k, do[0, rws, :], do[1, rws, :], +1))
                    t.append(_fft16_a(a4, n0, +1))
                    yield token(t[-1][1][0], t[-1][3][1], t[-1][0][0], t[-1][2][1])
                for k0 in range(4):
                    o = _radix4([t[n0][k0] for n0 in range(4)], +1)
                    for k1 in range(4):
                        n = k0 + 4 * k1
                        yr, yi = o[k1]
                        if g == 0:
                            yi = jnp.where(row8 + it == 0, nyb[n, dyn(0, 8), :], yi)
                        yp.at[n // 2][pl.ds(blk(it, 32, 8 * g), 8), (n % 2) * 128:(n % 2 + 1) * 128] = _pk2(yr, yi)
                    yield token(*[v for z in o for v in z])
        return Job(gen(), 32)

    def ny1_job():
        def gen():
            zero = jnp.zeros((8, 128), f32)
            t = []
            for n0 in range(4):
                t.append(_fft16_a([(x1[4 * n1 + n0, dyn(512, 8), :], zero) for n1 in range(4)], n0, -1))
                yield token(t[-1][1][0], t[-1][3][1], t[-1][0][0], t[-1][2][0])
            acc = [[zero, zero], [zero, zero]]
            for k0 in range(4):
                o = _radix4([t[n0][k0] for n0 in range(4)], -1)
                for k1 in range(4):
                    k = k0 + 4 * k1
                    v = twid(k, o[k1][0], o[k1][1], -1)
                    acc[k // 8] = [jnp.where(row8 == k % 8, v[e], acc[k // 8][e]) for e in range(2)]
                yield token(*acc[0], *acc[1])
            yield put3(lf, 0, *acc)
        return Job(gen(), 9)

    def ny_f():
        (xr, xi), = cdft(lf, 8, False)
        wr_ = _bf(wtr[0, dyn(256, 8), :]).astype(f32)
        wi_ = _bf(wti[0, dyn(256, 8), :]).astype(f32)
        yr, yi = cmul(xr, xi, wr_, wi_)
        put3(li, 0, (yr[0:8], yi[0:8]), (yr[8:16], yi[8:16]))

    def ny_i():
        (dr, di), = cdft(li, 8, True)
        do[0, 0:16, :] = dr
        do[1, 0:16, :] = di

    def ny3_job():
        def gen():
            t = []
            for n0 in range(4):
                a4 = []
                for n1 in range(4):
                    k = 4 * n1 + n0
                    re, im = (jnp.broadcast_to(do[e, pl.ds(zr[0] + k, 1), :], (8, 128)) for e in range(2))
                    a4.append(twid(k, re, im, +1))
                t.append(_fft16_a(a4, n0, +1))
                yield token(t[-1][1][0], t[-1][3][1], t[-1][0][0], t[-1][2][1])
            for k0 in range(4):
                o = _radix4([t[n0][k0] for n0 in range(4)], +1)
                for k1 in range(4):
                    nyb[k0 + 4 * k1] = o[k1][0]
                yield token(*[o[k1][0] for k1 in range(4)])
        return Job(gen(), 8)

    def si_tile(j, fused):
        def yk(r):
            return yp[j // 2, dyn(r, 64), (j % 2) * 128:(j % 2 + 1) * 128]

        e0 = _dot(_bf(yk(0)), _bf(cb[328:392, 0:128]), _TN)
        e2 = _dot(_bf(yk(128)), _bf(cb[328:392, 128:256]), _TN)
        y13 = jnp.concatenate([yk(64), yk(192)], axis=0)
        pq = _dot(_bf(y13), _bf(cb[200:328, :]), _TN)
        p, q = pq[:, 0:128], pq[:, 128:256]
        ep, em = e0 + e2, e0 - e2
        sync[0] = None
        st = jnp.concatenate([ep + p, em + q, ep - p, em - q], axis=1)
        rs = slice(j * 128, (j + 1) * 128)
        if fused:
            ob[rs, :] = (xb[rs, :].astype(f32) + st * gate[dyn(j * 128, 128), :]).astype(jnp.bfloat16)
        else:
            sbuf[j // 4] = st

    d0, d1 = dyn(0, MQ, 0), dyn(0, MQ, 1)

    def strassen(prod, bufs, out):
        put, get = bufs
        put(0, prod(0))
        yield
        m = prod(1)
        put(1, m)
        put(2, get(0, 0) - m)
        yield
        m = prod(2)
        put(3, m)
        put(4, get(2, 0) + m)
        yield
        out(1, 1, prod(3) + get(4, 0))
        yield
        m = prod(4)
        out(0, 1, get(3, 0) + m)
        put(5, get(0, 1) - m)
        yield
        m = prod(5)
        out(1, 0, get(1, 0) + m)
        put(6, get(5, 0) + m)
        yield
        out(0, 0, prod(6) + get(6, 0))
        yield

    def g_quad(q, jobs, after):
        cur = [0]
        vb_ = (va, vb, vc, vd, ve, vf, vg)
        ub_ = (ua, ub, uc, ud, ue, uf, ug)

        def prod(n, m):
            o = 7 * n + m
            lhs = jnp.concatenate(
                [sa[kt, o // 2, dyn(0, MQ // 2), (o % 2) * 128:(o % 2 + 1) * 128] for kt in range(4)], axis=1)
            if n in _RDIR and m in _RDIR:
                kq, tn = 2 * _RDIR[n][0] + _RDIR[m][0], 2 * _RDIR[n][1] + _RDIR[m][1]
                w = wspb[pl.ds(blk(q, 128, tn * KQ), 128), kq * KQ:(kq + 1) * KQ]
            else:
                t, ix = tslot(n, m)
                w = _bf(t[ix, dyn(0, 64), :])
            tk = spread(jobs.get(cur[0], []), 22)
            r = _dot(_bf(synced(lhs)), w, _NT)
            sync[0] = token(r[MQ - SYL:MQ - SYL + 8])
            return tiev(r, tk)

        def vput(k, v):
            vb_[k][0:MQ, :] = v

        def vget(k, w):
            return vb_[k][d1 if w else d0, :]

        def emit(half, tile, m2, tn, c):
            tq = tn + 2 * tile
            j = q + 4 * tq
            lo = half * MH + m2 * MQ
            n = min(MQ, FH - lo)
            hv = gelu2(y1s[j, dyn(lo, n), :]) * (c[0:n] + bbc[j, dyn(0, 8), :][0:1])
            h, hl = hlanes(tq)
            h[lo // 2:(lo + n) // 2, hl] = _pk(hv)

        def combine(n, m2, tn, m):
            s = 2 * m2 + tn

            def put(k, v):
                ub_[k][s, 0:MQ, :] = v

            def get(k, w):
                return ub_[k][s, d1 if w else d0, :]

            if n == 0:
                put(0, m)
            elif n == 1:
                put(1, m)
                put(2, get(0, 0) - m)
            elif n == 2:
                put(3, m)
                put(4, get(2, 0) + m)
            elif n == 3:
                emit(1, 1, m2, tn, m + get(4, 0))
            elif n == 4:
                emit(0, 1, m2, tn, get(3, 0) + m)
                put(5, get(0, 1) - m)
            elif n == 5:
                emit(1, 0, m2, tn, get(1, 0) + m)
                put(6, get(5, 0) + m)
            else:
                emit(0, 0, m2, tn, m + get(6, 0))

        for n in range(7):
            for _ in strassen(lambda m, n=n: prod(n, m), (vput, vget),
                              lambda i, j, v, n=n: combine(n, i, j, v)):
                for fn in after.get(cur[0], []):
                    fn()
                cur[0] += 1

    def tjobs(jobs, q, last=False):
        over(jobs, tprep_job(q, 1), 0, 27)
        if not last:
            over(jobs, tprep_job(q + 1, 0), 29, 49)

    jobs, after = {}, {}
    Q0 = CFG["q0"]
    over(jobs, wout_job(), *Q0["wo"])
    over(jobs, wprep_a_job(), *Q0["wa"])
    over(jobs, wprep_b_job(), *Q0["wb"])
    tjobs(jobs, 0)
    over(jobs, ny1_job(), *Q0["s1"])
    add(after, Q0["f"], ny_f)
    add(after, Q0["i"], ny_i)
    over(jobs, ny3_job(), *Q0["s3"])
    add(after, 37, lambda: o_tile(0, 2, False))
    add(after, 41, lambda: o_tile(0, 3, False))
    g_quad(0, jobs, after)
    wait(grp_4)

    def p2_body(it, carry):
        sync[0] = None
        q = 1 + it
        jobs, after = {}, {}
        for c in range(4):
            a1, b1, a3, b3 = CFG["fs"][c]
            over(jobs, s1_job(c, it), a1, b1 + 1)
            add(after, CFG["tf"][c], lambda c=c: f_op(c, it))
            add(after, CFG["tf"][c] + 3, i_op)
            over(jobs, s3_job(c, it), a3, b3 + 1)
        tjobs(jobs, q)
        add(after, 2, lambda: o_tile(q - 1, 0, False))
        add(after, 6, lambda: o_tile(q - 1, 1, False))
        add(after, 38, lambda: o_tile(q, 2, False))
        add(after, 43, lambda: o_tile(q, 3, False))
        g_quad(q, jobs, after)
        return carry

    jax.lax.fori_loop(0, 2, p2_body, 0)
    sync[0] = None

    outs = []

    def out_dma(lo, hi, bases=(0, 4, 8, 12)):
        for base in bases:
            outs.append(o_cp(base + lo, base + hi))
            outs[-1].start()

    jobs, after = {}, {}
    tjobs(jobs, 3, last=True)
    add(after, 2, lambda: o_tile(2, 0, False))
    add(after, 5, lambda: o_tile(2, 1, False))
    gated = [j for j in range(NB) if j % 4 != 3]
    for n in range(6):
        add(after, 7 + 3 * n, lambda n=n: (si_tile(gated[2 * n], True), si_tile(gated[2 * n + 1], True)))
    add(after, 26, lambda: (si_tile(3, False), si_tile(7, False)))
    add(after, 29, lambda: (si_tile(11, False), si_tile(15, False)))
    add(after, 31, lambda: out_dma(0, 3))
    add(after, 43, lambda: o_tile(3, 2, True))
    add(after, 48, lambda: o_tile(3, 3, True))
    g_quad(3, jobs, after)
    o_tile(3, 0, True)
    out_dma(3, 4, (8, 12))
    o_tile(3, 1, True)
    out_dma(3, 4, (0,))
    out_dma(3, 4, (4,))
    wait(outs)


@jax.jit
def pallas_recurrent_scan__spectral_gfnet__mixer_gmlp__prompt_kernel(
    A_x: jax.Array,
    A_w_r: jax.Array,
    A_w_i: jax.Array,
    B_x: jax.Array,
    B_w_in: jax.Array,
    B_w_sp: jax.Array,
    B_b_sp: jax.Array,
    B_w_out: jax.Array,
):
    del B_x
    bf16, f32, u32 = jnp.bfloat16, jnp.float32, jnp.uint32
    hbm_spec = pl.BlockSpec(memory_space=pltpu.HBM)
    scratch = [
        pltpu.VMEM((S, D), bf16),
        pltpu.VMEM((F, D), bf16),
        pltpu.VMEM((F // 2, D), u32),
        pltpu.VMEM((FH, D), bf16),
        pltpu.VMEM((FHP // 2, D), u32),
        pltpu.VMEM((S, S), bf16),
        pltpu.VMEM((4 * S,), bf16),
        pltpu.VMEM((NB, 32, 128), f32),
        pltpu.VMEM((257, S), bf16),
        pltpu.VMEM((257, S), bf16),
        pltpu.VMEM((2, S // 2, 128), u32),
        pltpu.VMEM((2, S // 2, 128), u32),
        pltpu.VMEM((S // 2, 128), u32),
        pltpu.VMEM((8, 264, 128), u32),
        pltpu.VMEM((8, 264, 128), u32),
        pltpu.VMEM((528, 256), u32),
        pltpu.VMEM(_TW.shape, f32),
        pltpu.VMEM((9, 64, 256), u32),
        pltpu.VMEM((9, 64, 256), u32),
        pltpu.VMEM((7, MH // 2, 256), u32),
    ] + [pltpu.VMEM((MH, 128), f32)] * 10 + [
    ] + [pltpu.VMEM((64, 768), u32)] * 4 + [
        pltpu.VMEM((2, 256, 128), f32),
        pltpu.VMEM((2, 256, 128), f32),
        pltpu.VMEM((32, 128), f32),
        pltpu.VMEM((32, 128), f32),
        pltpu.VMEM((NB, 544, 128), f32),
        pltpu.VMEM((NB, 2 * MH, 128), f32),
    ] + [pltpu.VMEM((2 * MH, 128), f32)] * 4 + [
        pltpu.VMEM((7, MH, 128), f32),
        pltpu.VMEM((4, 25, 96, 256), u32),
        pltpu.VMEM((28, 64, KQ), u32),
        pltpu.VMEM((21, 64, KQ), u32),
    ] + [pltpu.VMEM((4, 192, 128), f32)] * 7 + [
    ] + [pltpu.VMEM((192, 128), f32)] * 7 + [
    ] + [
        pltpu.VMEM((MH, 256), u32),
        pltpu.VMEM((MH, 256), u32),
        pltpu.VMEM((256, 384), u32),
        pltpu.VMEM((256, 384), u32),
        pltpu.VMEM((2, 512, 128), f32),
        pltpu.VMEM((NB, 8, 128), f32),
        pltpu.VMEM((NB // 2, 256, 256), u32),
        pltpu.VMEM((S, D), f32),
        pltpu.VMEM((4, 128, D), f32),
        pltpu.VMEM((S, D), bf16),
        pltpu.SMEM((8,), jnp.int32),
        pltpu.SemaphoreType.DMA((11,)),
    ]
    return pl.pallas_call(
        _kernel,
        in_specs=[hbm_spec] * 10,
        out_specs=hbm_spec,
        out_shape=jax.ShapeDtypeStruct(A_x.shape, A_x.dtype),
        scratch_shapes=scratch,
        compiler_params=pltpu.CompilerParams(vmem_limit_bytes=110 * 1024 * 1024),
    )(A_x, A_w_r.T, A_w_i.T, B_w_in.T, B_w_sp, B_b_sp, B_w_out, jnp.asarray(_CB), jnp.asarray(_TW),
      jnp.asarray(np.zeros((8,), np.int32)))
```

```python
import math

import jax
import jax.numpy as jnp
import numpy as np
import jax.experimental.pallas as pl
import jax.experimental.pallas.tpu as pltpu

S = 2048
D = 512
F = 1376
FH = 688
FHP = 768
NB = 16
NX = 528
EPS = 1e-5

_C = math.sqrt(2.0 / math.pi)
_A = 0.044715
KAPPA = (_C * _A) ** (1.0 / 3.0)
BETA = _C / KAPPA
EPS2 = 4.0 * KAPPA * KAPPA * EPS
INV4K = 1.0 / (4.0 * KAPPA)

_NT = (((1,), (1,)), ((), ()))
_NN = (((1,), (0,)), ((), ()))
_TN = (((0,), (0,)), ((), ()))


def _pack_rows(m):
    u = np.ascontiguousarray(m, dtype=np.float32).view(np.uint32).astype(np.uint64)
    b = ((u + 0x7FFF + ((u >> 16) & 1)) >> 16).astype(np.uint32)
    return b[0::2] | (b[1::2] << 16)


def _tables():
    n2 = np.arange(128)
    gf = np.zeros((4, 128, 256))
    mi = np.zeros((4, 128, 256))
    for c in range(4):
        for j in range(64):
            k = 4 * j + c
            th = 2 * np.pi * k * n2 / 512
            co, si = np.cos(th), np.sin(th)
            m, r = j // 8, j % 8
            re = 16 * m + r
            im = re + 8
            kre, kim = re, im
            w = 1.0 if k == 0 else 2.0
            if c in (0, 2):
                gf[c, re, :128], gf[c, im, :128] = co, -si
                mi[c, kre, :128], mi[c, kim, :128] = w * co, -w * si
            elif c == 1:
                gf[c, re, :128], gf[c, re, 128:] = co, -si
                gf[c, im, :128], gf[c, im, 128:] = -si, -co
                mi[c, kre, :128], mi[c, kim, :128] = w * co, -w * si
                mi[c, kre, 128:], mi[c, kim, 128:] = -w * si, -w * co
            else:
                gf[c, re, :128], gf[c, re, 128:] = co, si
                gf[c, im, :128], gf[c, im, 128:] = -si, co
                mi[c, kre, :128], mi[c, kim, :128] = w * co, -w * si
                mi[c, kre, 128:], mi[c, kim, 128:] = w * si, w * co
    nyq = np.cos(np.pi * n2)
    g0 = np.zeros((144, 128))
    g0[:128] = gf[0, :, :128]
    g0[128:136] = nyq
    g2 = np.zeros((144, 128))
    g2[:128] = gf[2, :, :128]
    mi[0, 8, :128] = nyq
    godd = np.zeros((256, 256))
    for n, c in enumerate((1, 3)):
        ks = 4 * np.arange(64) + c
        th = 2 * np.pi * np.outer(ks, n2) / 512
        godd[64 * n:64 * n + 64, :128] = np.cos(th) - np.sin(th)
        godd[64 * n:64 * n + 64, 128:] = (np.cos(th) + np.sin(th)) * (-1.0 if c == 1 else 1.0)
        godd[128:192, 128 * n:128 * n + 128] = np.cos(th)
    fs = 1.0 / KAPPA
    bs = 1.0 / (S * D)
    cc = np.cos(2 * np.pi * np.outer(n2, n2) / 128)
    ss = np.sin(2 * np.pi * np.outer(n2, n2) / 128)
    cb = np.concatenate(
        [
            godd * fs,
            np.concatenate([g0, g2], 1) * fs,
            mi[1] * bs,
            mi[3] * bs,
            np.concatenate([mi[0, :, :128], mi[2, :, :128]], 1) * bs,
            np.concatenate([cc, np.zeros((128, 128))], 1),
            np.concatenate([ss - cc, -ss - cc], 1),
        ],
        0,
    )
    k1 = np.arange(16)
    ph = 2 * np.pi * np.outer(k1, n2) / 2048
    tw = np.concatenate([np.cos(ph), np.sin(ph)], 1)
    tw = np.repeat(tw, 8, axis=0).astype(np.float32)
    return _pack_rows(cb), tw


_CB, _TW = _tables()


def _bf(u32):
    return pltpu.bitcast(u32, jnp.bfloat16)


def _u32(bf):
    return pltpu.bitcast(bf, jnp.uint32)


def _bits(f):
    return jax.lax.bitcast_convert_type(f, jnp.uint32)


def _dot(a, b, dims):
    return jax.lax.dot_general(a, b, dims, preferred_element_type=jnp.float32)


def _pk(v):
    return _u32(v.astype(jnp.bfloat16))


def _pk2(a, b):
    return _pk(jnp.concatenate([a, b], axis=0))


def _unpk(u):
    lo = jax.lax.bitcast_convert_type(u << 16, jnp.float32)
    hi = jax.lax.bitcast_convert_type(u & jnp.uint32(0xFFFF0000), jnp.float32)
    return lo, hi


def _radix4(a, sign):
    (ar, ai), (br, bi), (cr, ci), (dr, di) = a
    s0r, s0i = ar + cr, ai + ci
    d0r, d0i = ar - cr, ai - ci
    s1r, s1i = br + dr, bi + di
    d1r, d1i = br - dr, bi - di
    o0 = (s0r + s1r, s0i + s1i)
    o2 = (s0r - s1r, s0i - s1i)
    if sign < 0:
        o1 = (d0r + d1i, d0i - d1r)
        o3 = (d0r - d1i, d0i + d1r)
    else:
        o1 = (d0r - d1i, d0i + d1r)
        o3 = (d0r + d1i, d0i - d1r)
    return [o0, o1, o2, o3]


def _tw16(x, e, sign):
    e = e % 16
    xr, xi = x
    if e == 0:
        return x
    if e == 4:
        return (xi, -xr) if sign < 0 else (-xi, xr)
    if e in (2, 6):
        h = math.sqrt(0.5)
        if e == 2:
            if sign < 0:
                return ((xr + xi) * h, (xi - xr) * h)
            return ((xr - xi) * h, (xi + xr) * h)
        if sign < 0:
            return ((xi - xr) * h, (xr + xi) * (-h))
        return ((xr + xi) * (-h), (xr - xi) * h)
    ang = sign * 2 * math.pi * e / 16
    wr, wi = math.cos(ang), math.sin(ang)
    return (xr * wr - xi * wi, xr * wi + xi * wr)


def _fft16_a(a4, n0, sign):
    o = _radix4(a4, sign)
    return [_tw16(o[k0], n0 * k0, sign) for k0 in range(4)]


MH = 352
MQ = 176
KQ = S // 4
SYL = 144

CFG = dict(
    q0=dict(wo=[1, 7], wa=[8, 21], wb=[22, 48], s1=[8, 20], f=28, i=31, s3=[34, 44]),
    tf=[5, 14, 23, 32], fs=[[0, 4, 10, 13], [6, 9, 19, 22], [15, 18, 28, 36], [24, 27, 39, 48]],
    lsn=0, l2r=[0, 7], lnw=24, lnb=8, win=5, tz2=[0, 0, 8, 16], tz1=[6, 6, 6, 6, 0, 0, 0],
)


def _str_l(a11, a12, a21, a22):
    if a22 is None:
        return (a11, a21, a11, -a11 if a21 is None else a21 - a11, a11 + a12, None, a12)
    return (a11 + a22, a21 + a22, a11, a21 - a11, a11 + a12, a22, a12 - a22)


def _str_r(b11, b21, b12, b22):
    return (b11 + b22, b11, b12 - b22, b11 + b12, b22, b21 - b11, b21 + b22)


_SUMS_L, _SUMS_R = (0, 1, 3, 4, 6), (0, 2, 3, 5, 6)
_RDIR = {1: (0, 0), 4: (1, 1)}


def _kernel(
    x_hbm, wr_hbm, wi_hbm, win_hbm, wsp_hbm, b_hbm, wout_hbm, cb_hbm, tw_hbm, z_hbm,
    o_hbm,
    xb, winb, wint, woutb, woutp, wspb, bb, bbc, wrb, wib, w32r, w32i, w32n, wtr, wti,
    cb, tw, xs0, xs1, wz, qa, qb, qc, qd, qe, qf, qg, qh, qi, qj, ys0, ys1, ys2, ys3, ls0, ls1, st_m, st_r,
    x1, y1s, zf0, zf1, zf2, zf3, xa0, sa, tbx, tby, ua, ub, uc, ud, ue, uf, ug, va, vb, vc, vd, ve, vf, vg,
    hlo, hhi, lf, li, do, nyb, yp, gate, sbuf, ob, zs, sems,
):
    f32, u32 = jnp.float32, jnp.uint32
    nsem = [0]

    def cp(src, dst):
        return pltpu.make_async_copy(src, dst, sems.at[nsem[0]])

    def group(*cps):
        nsem[0] += 1
        return [c for x in cps for c in (x if isinstance(x, list) else [x])]

    def rows(ref, lo, hi):
        return ref.at[pl.ds(lo, hi - lo), :]

    def xcp(lo, hi):
        return cp(x_hbm.at[0, pl.ds(lo * 128, (hi - lo) * 128), :], rows(xb, lo * 128, hi * 128))

    def wspcp(lo, hi):
        return [cp(rows(wsp_hbm, h + lo, h + hi), rows(wspb, h + lo, h + hi)) for h in (0, KQ, 2 * KQ, 3 * KQ)]

    def o_cp(lo, hi):
        return cp(rows(ob, lo * 128, hi * 128), o_hbm.at[0, pl.ds(lo * 128, (hi - lo) * 128), :])

    grp_z = group(cp(z_hbm, zs))
    grp_a = group(xcp(0, 1))
    grp_b = group(xcp(8, 9), cp(rows(win_hbm, FH, FH + MH), rows(winb, FH, FH + MH)))
    grp_c = group(cp(rows(win_hbm, FH + MH, F), rows(winb, FH + MH, F)), xcp(4, 5), xcp(12, 13))
    grp_d = group(cp(rows(win_hbm, 0, FH), rows(winb, 0, FH)), cp(rows(cb_hbm, 0, 200), rows(cb, 0, 200)),
                  xcp(1, 2), xcp(9, 10))
    grp_1 = group(xcp(5, 6), xcp(13, 14), xcp(2, 3), xcp(10, 11), wspcp(0, 48))
    grp_2 = group(xcp(6, 8), xcp(14, 16), xcp(3, 4), xcp(11, 12), wspcp(48, 128))
    grp_3 = group(wspcp(128, 256), cp(wr_hbm, wrb), cp(wi_hbm, wib), cp(wout_hbm, woutb),
                  cp(rows(cb_hbm, 200, 520), rows(cb, 200, 520)), cp(tw_hbm, tw))
    grp_3 += group(cp(b_hbm, bb.at[pl.ds(0, S)]))
    grp_4 = group(wspcp(256, 512))

    def wait(grp):
        for c_ in grp:
            c_.wait()

    for c_ in grp_z + grp_a + grp_b + grp_c + grp_d + grp_1 + grp_2 + grp_3 + grp_4:
        c_.start()
    wait(grp_z + grp_a)

    zr = [zs[n] for n in range(3)]
    zvec = jnp.full((8, 128), zr[2], jnp.int32).astype(u32)

    def dyn(lo, n, w=0, stride=None):
        if stride is None:
            return pl.ds(pl.multiple_of(zr[w] + lo, 8), n)
        return pl.ds(zr[w] + lo, n, stride=stride)

    def blk(i, n, extra=0):
        if isinstance(i, int):
            return i * n + extra
        return pl.multiple_of(i * n + extra, 8)

    def token(*vs):
        acc = None
        for v in vs:
            if v.dtype != u32:
                v = _bits(v)
            for r in range(0, v.shape[0], 8):
                for c in range(0, v.shape[1], 128):
                    t = v[r:r + 8, c:c + 128]
                    acc = t if acc is None else acc | t
        return acc

    def htoken(*vs):
        return token(*[v[r:r + 8] for v in vs[0::2] for r in range(8, v.shape[0], 16)])

    sync = [None]

    def synced(u):
        if sync[0] is None:
            return u
        sz = sync[0] & zvec
        cols = [u[0:8, c:c + 128] | sz for c in range(0, u.shape[1], 128)]
        return jnp.concatenate([jnp.concatenate(cols, axis=1), u[8:]], axis=0)

    def tiev(v, toks):
        parts = []
        prev = 0
        for r in sorted(toks):
            if r * 8 > prev:
                parts.append(v[prev:r * 8])
            parts.append(jax.lax.bitcast_convert_type(_bits(v[r * 8:r * 8 + 8]) | (toks[r] & zvec), f32))
            prev = r * 8 + 8
        if prev < v.shape[0]:
            parts.append(v[prev:])
        return jnp.concatenate(parts, axis=0) if len(parts) > 1 else parts[0]

    ALL = 9999
    rel = [None]

    def gate_(v):
        if rel[0] is None:
            return v
        u = v if v.dtype == u32 else _bits(v)
        tiles = [[u[r:r + 8, c:c + 128] | rel[0] for c in range(0, u.shape[1], 128)]
                 for r in range(0, u.shape[0], 8)]
        u = jnp.concatenate([jnp.concatenate(t, axis=1) for t in tiles], axis=0)
        return u if v.dtype == u32 else jax.lax.bitcast_convert_type(u, v.dtype)

    class Job:
        def __init__(self, gen, n, win=None):
            self.gen, self.left, self.win = gen, n, CFG["win"] if win is None else win

        def __next__(self):
            self.left -= 1
            return next(self.gen)

    def spread(lists, nslot, src=None):
        out = {}
        rels = {}
        for job, n, lo, hi in lists:
            n = min(n, job.left)
            for k in range(n):
                sl = min(int(nslot * (lo + (k + 0.5) * (hi - lo) / n)), nslot - 1)
                rs = sl - job.win
                if src is not None and rs >= 0:
                    if rs not in rels:
                        rels[rs] = _bits(src[8 * rs:8 * rs + 8]) & zvec
                    rel[0] = rels[rs]
                tk = next(job)
                rel[0] = None
                out[sl] = tk if sl not in out else out[sl] | tk
        return out

    def add(d, k, v):
        d.setdefault(k, []).append(v)

    def over(jobs, job, lo, hi):
        n = -(-job.left // (hi - lo))
        for pos in range(lo, hi):
            add(jobs, pos, (job, n if pos < hi - 1 else ALL, 0.0, 1.0))

    xsb, ysb, zfb = (xs0, xs1), (ys0, ys1, ys2, ys3), (zf0, zf1, zf2, zf3)
    TOFF = (0, 8, 4, 12)
    row8 = jax.lax.broadcasted_iota(jnp.int32, (8, 128), 0)

    def ln_stats(x):
        m = jnp.sum(x, axis=-1, keepdims=True) * (1.0 / D)
        v = jnp.sum(x * x, axis=-1, keepdims=True) * (1.0 / D) - m * m
        return m, jax.lax.rsqrt(jnp.maximum(v, 0.0) + EPS) * KAPPA

    def xrows(i, r):
        return xb[pl.ds(blk(i, 128, r), 16), :].astype(f32)

    def lns_job(i, p):
        def gen():
            for r in range(0, 128, 16):
                for e in range(2):
                    x = gate_(xrows(i + 8 * e, r))
                    sts = [ln_stats(x[8 * hf:8 * hf + 8]) for hf in range(2)]
                    st = [jnp.broadcast_to(sts[hf][n], (8, 128)) for n in range(2) for hf in range(2)]
                    for n, v in enumerate(st):
                        (ls1 if p else ls0)[e, 2 * r + 8 * n:2 * r + 8 * n + 8, :] = v
                    yield token(*st)
        return Job(gen(), 16, CFG["lnw"])

    def ln_rows(i, b, r, pre=False):
        if pre:
            x = xrows(i, r)
            ls = ls1 if b // 2 else ls0
            m, rs = gate_(ls[b % 2, dyn(2 * r, 16), :]), ls[b % 2, dyn(2 * r + 16, 16), :]
            a0, a1, a2, a3 = ((x[:, 128 * j:128 * (j + 1)] - m) * rs for j in range(4))
            xn = jnp.concatenate([a0, a1, a2, a3], axis=1)
        else:
            x = gate_(xrows(i, r))
            m, rs = ln_stats(x)
            xn = (x - m) * rs
            a0, a1, a2, a3 = (xn[:, 128 * j:128 * (j + 1)] for j in range(4))
        s02, s13 = a0 + a2, a1 + a3
        p, q = a0 - a2, a1 - a3
        ys = [s02 + s13, s02 - s13, p, q, p + q, p - q]
        ysb[b][r // 2:r // 2 + 8, :] = _pk(jnp.concatenate(ys, axis=1))
        for hf in range(2):
            xsb[b // 2].at[PLAIN[b % 2][hf]][r // 2:r // 2 + 8, :] = _pk(xn[:, 256 * hf:256 * (hf + 1)])
        return xn, htoken(ys[0], ys[1], ys[4], ys[5])

    PLAIN = ((1, 7), (8, 4))

    def ln_job(i, b):
        def gen():
            for r in range(0, 128, 16):
                yield ln_rows(i, b, r)[1]
        return Job(gen(), 8, CFG["lnw"])

    def lnp_job(i, p, win=None, pre=True):
        def gen():
            for r in range(0, 128, 16):
                a, tk = ln_rows(i, 2 * p, r, pre)
                yield tk
                b, tk = ln_rows(i + 8, 2 * p + 1, r, pre)
                ops = _str_r(a[:, 0:256], a[:, 256:512], b[:, 0:256], b[:, 256:512])
                for n in _SUMS_R:
                    xsb[p].at[n][r // 2:r // 2 + 8, :] = _pk(ops[n])
                yield tk | htoken(*[ops[n] for n in _SUMS_R])
        return Job(gen(), 16, CFG["lnw"] if win is None else win)

    def wz_job():
        def ld(r, lanes):
            return gate_(winb[r:r + 16, lanes].astype(f32))

        def gen():
            for r in range(0, MH, 16):
                for c in range(2):
                    lo, hi = slice(c * 128, (c + 1) * 128), slice(256 + c * 128, 256 + (c + 1) * 128)
                    a11, a12 = ld(r, lo), ld(r, hi)
                    bot = (ld(MH + r, lo), ld(MH + r, hi)) if MH + r < FH else (None, None)
                    ops = _str_l(a11, a12, *bot)
                    for n in range(7):
                        if ops[n] is None:
                            wz.at[n][r // 2:r // 2 + 8, lo] = jnp.zeros((8, 128), u32)
                        else:
                            wz.at[n][r // 2:r // 2 + 8, lo] = _pk(ops[n])
                    yield token(*[ops[n] for n in _SUMS_L if ops[n] is not None])
        return Job(gen(), 44)

    def gelu2(z):
        return z + z * jnp.tanh(z * (z * z + BETA))

    def cdot(r0, r1, lanes, w):
        outs = []
        r = r0
        while r < r1:
            n = min(64, r1 - r)
            if r1 - r - n == 16:
                n += 16
            outs.append(_dot(_bf(cb[r // 2:(r + n) // 2, lanes]), w, _NT))
            r += n
        return jnp.concatenate(outs, axis=0)

    L0, L1 = slice(0, 128), slice(128, 256)

    def l1_job(kq):
        xa = xa0
        G = 32

        def nrm(e, lo, n, mg):
            z = zfb[2 * kq + e][dyn(lo, n, 1), :].reshape(n // 8, 8, 128)
            return ((z - mg[e]) * st_r[dyn(8 * (2 * kq + e), 8), :]).reshape(n, 128)

        def gen():
            for r in range(0, MH, G):
                n2 = min(G, FH - MH - r)
                mg = [gate_(st_m[dyn(8 * (2 * kq + e), 8), :]) for e in range(2)]
                top = [nrm(e, r, G, mg) for e in range(2)]
                bot = [nrm(e, MH + r, n2, mg) for e in range(2)]
                if n2 < G:
                    pad = jnp.zeros((G - n2, 128), f32)
                    bot = [jnp.concatenate([v, pad], axis=0) for v in bot]
                ops = _str_l(top[0], top[1], bot[0], bot[1])
                for n, v in enumerate(ops):
                    xa[n, r:r + G, :] = v
                yield htoken(*[ops[n] for n in _SUMS_L])
        return Job(gen(), 11)

    def l2_job(kt):
        def gen():
            for r in range(0, MQ, 16):
                zn = {}
                for e in range(2):
                    m, rs = gate_(st_m[dyn(8 * (2 + e), 8), :]), st_r[dyn(8 * (2 + e), 8), :]
                    for qd_ in range(4):
                        lo = qd_ * MQ + r
                        if lo < FH:
                            z = zfb[2 + e][dyn(lo, 16, 1), :].reshape(2, 8, 128)
                            zn[e, qd_] = ((z - m) * rs).reshape(16, 128)
                        else:
                            zn[e, qd_] = None
                l1 = [_str_l(zn[0, m2], zn[1, m2], zn[0, 2 + m2], zn[1, 2 + m2]) for m2 in range(2)]
                for n in range(7):
                    ops = _str_l(gate_(xa0[n, dyn(r, 16), :]), l1[0][n], xa0[n, dyn(MQ + r, 16), :], l1[1][n])
                    for m, v in enumerate(ops):
                        o = 7 * n + m
                        sa.at[kt, o // 2][r // 2:r // 2 + 8, (o % 2) * 128:(o % 2 + 1) * 128] = (
                            jnp.zeros((8, 128), u32) if v is None else _pk(v))
                    yield htoken(*[ops[m] for m in _SUMS_L])
        return Job(gen(), 77)

    def wprep_a_job():
        def gen():
            for b in range(NB):
                lanes = slice(b * 128, (b + 1) * 128)
                rws = slice(64 * b, 64 * (b + 1))
                for src, w32 in ((wrb, w32r), (wib, w32i)):
                    for j in range(2):
                        v = _u32(src[j * 128:(j + 1) * 128, lanes].T)
                        w32[j, rws, :] = v
                        yield token(v)
                nr, ni = (jnp.broadcast_to(src[256:257, lanes].astype(f32), (8, 128)) for src in (wrb, wib))
                slab = [jnp.where(row8 == 0, v, 0.0) for v in (nr, ni)] + [jnp.zeros((112, 128), f32)]
                v = _u32(jnp.concatenate(slab, axis=0).astype(jnp.bfloat16).T)
                w32n[rws, :] = v
                yield token(v)
        return Job(gen(), 80)

    def wprep_b_job():
        def gen():
            for r0 in range(8):
                tt = w32n[dyn(r0, 128, 0, 8), :].T[0:16]
                wtr[0, 256 + r0:257 + r0, :] = tt[0:1]
                wti[0, 256 + r0:257 + r0, :] = tt[8:9]
                yield token(tt)
            for r0 in range(8):
                for w32, wt in ((w32r, wtr), (w32i, wti)):
                    for j in range(2):
                        tt = w32[j, dyn(r0, 128, 0, 8), :].T
                        wt[r0, j * 128:(j + 1) * 128, :] = tt
                        yield token(tt)
        return Job(gen(), 40)

    def wout_job():
        def gen():
            woutp[FH // 2:FHP // 2, :] = jnp.zeros(((FHP - FH) // 2, D), u32)
            bvec = (bb[0:S].astype(f32) * INV4K).reshape(1, S)
            for j in range(NB):
                bbc[j, 0:8, :] = jnp.broadcast_to(bvec[:, j * 128:(j + 1) * 128], (8, 128))
            for c in range(4):
                lanes = slice(c * 128, (c + 1) * 128)
                for lo in range(0, FH, 64):
                    hi = min(lo + 64, FH)
                    v = _u32(woutb[lo:hi, lanes])
                    woutp[lo // 2:hi // 2, lanes] = v
                    yield token(v)
        return Job(gen(), 44)

    def tslot(n, m):
        return (tbx, 7 * n + m) if n < 4 else (tby, 7 * (n - 4) + m)

    def tprep_job(q, part, r_lo=0, nr=8):
        def gen():
            for rr in range(nr):
                r = r_lo + rr
                if not isinstance(r, int):
                    r = jnp.minimum(r, 7)
                ro = pl.ds(blk(r, 8), 8)
                for c in range(4):
                    lanes = slice(c * 128, (c + 1) * 128)

                    def up(tn, kq):
                        base = blk(q, 128, tn * KQ) + blk(r, 16)
                        if not isinstance(base, int):
                            base = pl.multiple_of(base, 16)
                        return gate_(wspb[pl.ds(base, 16), kq * KQ + c * 128:kq * KQ + (c + 1) * 128].astype(f32))

                    def level2(n, y):
                        ops = _str_r(y[0, 0], y[1, 0], y[0, 1], y[1, 1])
                        for m in range(7):
                            if n in _RDIR and m in _RDIR:
                                continue
                            t, ix = tslot(n, m)
                            t.at[ix][ro, lanes] = _pk(ops[m])
                        return htoken(*[ops[m] for m in _SUMS_R])

                    def cmb(a, b, sg):
                        return {k: a[k] + b[k] if sg > 0 else a[k] - b[k] for k in a}

                    def blk4(tn0, kq0):
                        return {(kq, tn): up(tn0 + tn, kq0 + kq) for kq in range(2) for tn in range(2)}

                    if part == 0:
                        b11 = blk4(0, 0)
                        yield level2(1, b11)
                        b22 = blk4(2, 2)
                        yield level2(0, cmb(b11, b22, 1))
                        b12 = blk4(2, 0)
                        yield level2(2, cmb(b12, b22, -1))
                        yield level2(3, cmb(b11, b12, 1))
                    else:
                        b22 = blk4(2, 2)
                        yield level2(4, b22)
                        b21 = blk4(0, 2)
                        yield level2(6, cmb(b21, b22, 1))
                        yield level2(5, cmb(b21, blk4(0, 0), -1))
        return Job(gen(), nr * 4 * (4 - part))

    def xplain(b, w):
        return _bf(jnp.concatenate([xsb[b // 2][n, dyn(0, 64, w), :] for n in PLAIN[b % 2]], axis=1))

    def z2_sink(b, lo, z, tk, st):
        CH = 4
        ng = z.shape[0] // 8
        marks = []
        for r in range(0, ng, CH):
            n = min(CH, ng - r)
            tkc = {k - r: v for k, v in tk.items() if r <= k < r + n}
            if len(marks) >= 2:
                tkc[0] = marks[-2] if 0 not in tkc else tkc[0] | marks[-2]
            y = gelu2(tiev(z[8 * r:8 * (r + n)], tkc))
            zfb[b][lo + 8 * r:lo + 8 * (r + n), :] = y
            for q in range(n):
                if "c" not in st:
                    st["c"] = y[0:8]
                    continue
                d = y[8 * q:8 * q + 8] - st["c"]
                st["sm"] = d if "sm" not in st else st["sm"] + d
                st["sq"] = d * d if "sq" not in st else st["sq"] + d * d
            marks.append(token(st["sm"], st["sq"]))
        st["n"] = st.get("n", 0) + ng
        if st["n"] == FH // 8:
            c, sm, sq, cnt = st["c"], st["sm"], st["sq"], FH // 8
            m2 = jnp.sum(sm + cnt * c, axis=0, keepdims=True) * (1.0 / FH)
            e = m2 - c
            v2 = jnp.sum(sq - 2.0 * e * sm + cnt * (e * e), axis=0, keepdims=True) * (1.0 / FH)
            st_m[8 * b:8 * b + 8, :] = jnp.broadcast_to(m2, (8, 128))
            st_r[8 * b:8 * b + 8, :] = jnp.broadcast_to(
                jax.lax.rsqrt(jnp.maximum(v2, 0.0) + EPS2) * INV4K, (8, 128))

    def z2_op(b, la, gated=True):
        z = _dot(_bf(wint[dyn(0, FH // 2), :]), xplain(b, 0), _NT)
        z2_sink(b, 0, z, spread(la, 86, z if gated else None), {})

    dq0, dq1 = dyn(0, MH, 0), dyn(0, MH, 1)

    def z1_chains(kt, jobs):
        rnd = [0]
        tks = []

        def pr(p, n):
            return _dot(_bf(synced(wz[n, dyn(0, MH // 2), :])), _bf(xsb[p][n, dyn(0, 64, 1), :]), _NT)

        def two(a, b):
            ra, rb = pr(*a), pr(*b)
            tks[:] = [spread(jobs.get(rnd[0], []), 42, ra)]
            sync[0] = token(ra[MH - SYL:MH - SYL + 8], rb[MH - SYL:MH - SYL + 8])
            rnd[0] += 1
            return ra, rb

        def tie1(v):
            return tiev(v, tks.pop()) if tks else v

        def out(b, lo, v):
            v = v[0:min(MH, FH - lo)]
            y1s[kt + TOFF[b], lo:lo + v.shape[0], :] = tie1(v)

        m1, m2 = two((0, 0), (0, 1))
        qa[...] = tie1(m1)
        qb[...] = m2
        qc[...] = m1 - m2
        m3, m6 = two((0, 2), (0, 3))
        out(1, MH, qc[dq0, :] + m3 + m6)
        qd[...] = m3
        m5, m4 = two((0, 4), (0, 5))
        out(1, 0, qd[dq0, :] + m5)
        out(0, MH, qb[dq0, :] + m4)
        qe[...] = qa[dq0, :] + m4 - m5
        m7, m1 = two((0, 6), (1, 0))
        out(0, 0, qe[dq0, :] + m7)
        qf[...] = m1
        m2, m3 = two((1, 1), (1, 2))
        qg[...] = tie1(m2)
        qh[...] = m3
        qi[...] = qf[dq0, :] - m2 + m3
        m6, m5 = two((1, 3), (1, 4))
        out(3, MH, qi[dq0, :] + m6)
        out(3, 0, qh[dq0, :] + m5)
        qj[...] = qf[dq1, :] - m5
        m4, m7 = two((1, 5), (1, 6))
        out(2, MH, qg[dq0, :] + m4)
        out(2, 0, qj[dq0, :] + m4 + m7)

    def d_op(i, b):
        y0, y2, p, q, pp, pm = (_bf(ysb[b][dyn(0, 64), 128 * n:128 * (n + 1)]) for n in range(6))
        o0 = cdot(256, 400, L0, y0)
        x1[i, 0:128, :] = o0[0:128]
        x1[i, 512:520, :] = o0[128:136]
        x1[i, 256:384, :] = cdot(256, 384, L1, y2)
        for n, (base, w) in enumerate(((128, pp), (384, pm))):
            t = cdot(128, 192, (L0, L1)[n], w)
            re = t + cdot(64 * n, 64 * n + 64, L1, q)
            im = cdot(64 * n, 64 * n + 64, L0, p) - t
            for m in range(8):
                x1[i, base + 16 * m:base + 16 * m + 8, :] = re[8 * m:8 * m + 8]
                x1[i, base + 16 * m + 8:base + 16 * m + 16, :] = im[8 * m:8 * m + 8]

    def p1_start():
        sts = [{}, {}]

        def z2_part(b, lo, hi, la):
            if b == 0:
                cols = []
                for c in range(4):
                    lanes = slice(c * 128, (c + 1) * 128)
                    cols.append(_u32(winb[FH + lo:FH + hi, lanes]))
                    wint[lo // 2:hi // 2, lanes] = cols[-1]
                lhs = jnp.concatenate(cols, axis=1)
            else:
                lhs = wint[dyn(lo // 2, (hi - lo) // 2), :]
            z = _dot(_bf(lhs), xplain(b, lo // MH), _NT)
            z2_sink(b, lo, z, spread(la, (hi - lo) // 8), sts[b])

        def z1_op(b, lb):
            if b == 0:
                cols = []
                for c in range(4):
                    lanes = slice(c * 128, (c + 1) * 128)
                    cols.append(_u32(winb[0:FH, lanes]))
                    wint[FH // 2:FH, lanes] = cols[-1]
                lhs = jnp.concatenate(cols, axis=1)
            else:
                lhs = wint[dyn(FH // 2, FH // 2), :]
            z = _dot(_bf(lhs), xplain(b, 1), _NT)
            y1s[TOFF[b], 0:FH, :] = tiev(z, spread(lb, 86, z))
            d_op(TOFF[b], b)

        lnj = ln_job(0, 0)
        while lnj.left:
            next(lnj)
        wait(grp_b)
        z2_part(0, 0, MH, [(ln_job(8, 1), ALL, 0.0, 0.6)])
        z2_part(1, 0, MH, [])
        wait(grp_c)
        ln4 = ln_job(4, 2)
        z2_part(0, MH, FH, [(ln4, 5, 0.0, 1.0)])
        z2_part(1, MH, FH, [(ln4, ALL, 0.0, 0.5)])
        z2_op(2, [(ln_job(12, 3), ALL, 0.0, 0.7)])
        z2_op(3, [(l1_job(0), ALL, 0.2, 1.0)])
        wait(grp_d)
        wzj, l2j, lnj = wz_job(), l2_job(0), lnp_job(1, 0, None, False)
        z1_op(0, [(l2j, 25, 0.0, 1.0), (wzj, 22, 0.0, 1.0)])
        z1_op(1, [(l2j, 25, 0.0, 1.0), (wzj, ALL, 0.0, 1.0)])
        z1_op(2, [(lnj, 8, 0.0, 1.0), (l2j, 14, 0.0, 1.0)])
        z1_op(3, [(lnj, ALL, 0.0, 0.8), (l2j, ALL, 0.0, 1.0)])

    def p1_quad(kt, bg):
        nk = jnp.minimum(kt + 1, 3)
        tz = CFG["tz2"]
        lnj = lnp_job(kt + 4, 1, CFG["lnb"])
        lsn = lns_job(nk, 0)
        z2_op(0, [(lns_job(kt + 4, 1), ALL, 0.0, 0.6), (lnj, 3, 0.75, 1.0), (bg, tz[0], 0.0, 1.0)])
        z2_op(1, [(lnj, ALL, 0.0, 0.8), (bg, tz[1], 0.0, 1.0)])
        z2_op(2, [(bg, tz[2], 0.0, 1.0), (l1_job(0), ALL, 0.2, 1.0)])
        z2_op(3, [(bg, tz[3], 0.0, 1.0), (lsn, CFG["lsn"], 0.0, 1.0)])
        d_op(kt, 0)
        d_op(kt + 8, 1)
        jobs = {}
        over(jobs, l2_job(kt), *CFG["l2r"])
        if lsn.left:
            over(jobs, lsn, 0, 4)
        over(jobs, lnp_job(nk, 0, CFG["lnb"]), 4, 7)
        for rn, n in enumerate(CFG["tz1"]):
            add(jobs, rn, (bg, n, 0.0, 1.0))
        z1_chains(kt, jobs)
        assert bg.left == 0
        d_op(kt + 4, 2)
        d_op(kt + 12, 3)

    p1_start()
    wait(grp_1)

    def p1_body(it, carry):
        @pl.when(it == 1)
        def _():
            wait(grp_2)

        sync[0] = None
        p1_quad(1 + it, tprep_job(0, 0, 3 * it, 3))
        return carry

    jax.lax.fori_loop(0, 3, p1_body, 0)
    sync[0] = None
    wait(grp_3)

    def hlanes(tn):
        return (hhi if tn // 2 else hlo), slice((tn % 2) * 128, (tn % 2 + 1) * 128)

    def o_tile(q, tn, fused):
        rs = pl.ds(blk(q, 128, tn * KQ), 128)
        h, hl = hlanes(tn)
        hp = jnp.concatenate([h[dyn(0, FH // 2), hl], jnp.zeros(((FHP - FH) // 2, 128), u32)], axis=0)
        w = _dot(_bf(hp), _bf(woutp[dyn(0, FHP // 2), :]), _TN)
        g = w + w * jnp.tanh(w)
        sync[0] = None
        if fused:
            ob[rs, :] = (xb[rs, :].astype(f32) + sbuf[tn, dyn(0, 128), :] * g).astype(jnp.bfloat16)
        else:
            gate[rs, :] = g

    def twid(k, re, im, sign):
        if k == 0:
            return re, im
        c = tw[8 * k:8 * k + 8, 0:128]
        s = tw[8 * k:8 * k + 8, 128:256]
        if sign < 0:
            return re * c + im * s, im * c - re * s
        return re * c - im * s, im * c + re * s

    def put3(dst, r0, a, b):
        sa_, sb_ = a[0] + a[1], b[0] + b[1]
        for n, (u, v) in enumerate(((sa_, sb_), (a[1], b[1]), (a[0], b[0]))):
            dst[r0:r0 + 8, 128 * n:128 * (n + 1)] = _pk2(u, v)
        return token(sa_, sb_)

    def s1_job(c, it):
        def gen():
            for gi in range(4):
                g = 8 * c + gi
                t = []
                for n0 in range(4):
                    a4 = [(x1[4 * n1 + n0, dyn(64 * it + 16 * g, 8), :],
                           x1[4 * n1 + n0, dyn(64 * it + 16 * g + 8, 8), :]) for n1 in range(4)]
                    t.append(_fft16_a(a4, n0, -1))
                    yield token(t[-1][1][0], t[-1][3][1], t[-1][0][0], t[-1][2][1])
                for kp in range(2):
                    oa = _radix4([t[n0][2 * kp] for n0 in range(4)], -1)
                    ob_ = _radix4([t[n0][2 * kp + 1] for n0 in range(4)], -1)
                    for k1 in range(4):
                        k = 4 * k1 + 2 * kp
                        yield put3(lf, 64 * gi + 4 * k, twid(k, *oa[k1], -1), twid(k + 1, *ob_[k1], -1))
        return Job(gen(), 48)

    def cdft(src, nrow, swap):
        m1 = _bf(cb[392:456, 0:128])
        m2 = _bf(cb[456:520, 0:128])
        m3 = _bf(cb[456:520, 128:256])
        if swap:
            m2, m3 = m3, m2
        n = max(nrow // 4, 8)
        for r in range(0, nrow, n):
            t1 = _dot(_bf(src[dyn(r, n), 0:128]), m1, _NN)
            yield (t1 + _dot(_bf(src[dyn(r, n), 128:256]), m2, _NN),
                   t1 + _dot(_bf(src[dyn(r, n), 256:384]), m3, _NN))
        sync[0] = None

    def cmul(xr, xi, wr_, wi_):
        return xr * wr_ - xi * wi_, xr * wi_ + xi * wr_

    def f_op(c, it):
        for gi, (xr, xi) in enumerate(cdft(lf, 256, False)):
            rws = dyn(32 * gi + c + 128 * it, 8, 0, 4)
            for pr in range(8):
                wr_, wi_ = _unpk(wtr[pr, rws, :]), _unpk(wti[pr, rws, :])
                ys = [cmul(xr[16 * pr + 8 * e:16 * pr + 8 * e + 8], xi[16 * pr + 8 * e:16 * pr + 8 * e + 8],
                           wr_[e], wi_[e]) for e in range(2)]
                put3(li, 64 * gi + 8 * pr, *ys)

    def i_op():
        for gi, (dr, di) in enumerate(cdft(li, 256, True)):
            do[0, 128 * gi:128 * (gi + 1), :] = dr
            do[1, 128 * gi:128 * (gi + 1), :] = di

    def s3_job(c, it):
        def gen():
            for gi in range(4):
                g = 8 * c + gi
                t = []
                for n0 in range(4):
                    a4 = []
                    for n1 in range(4):
                        k = 4 * n1 + n0
                        rws = dyn(128 * gi + 8 * k, 8)
                        a4.append(twid(k, do[0, rws, :], do[1, rws, :], +1))
                    t.append(_fft16_a(a4, n0, +1))
                    yield token(t[-1][1][0], t[-1][3][1], t[-1][0][0], t[-1][2][1])
                for k0 in range(4):
                    o = _radix4([t[n0][k0] for n0 in range(4)], +1)
                    for k1 in range(4):
                        n = k0 + 4 * k1
                        yr, yi = o[k1]
                        if g == 0:
                            yi = jnp.where(row8 + it == 0, nyb[n, dyn(0, 8), :], yi)
                        yp.at[n // 2][pl.ds(blk(it, 32, 8 * g), 8), (n % 2) * 128:(n % 2 + 1) * 128] = _pk2(yr, yi)
                    yield token(*[v for z in o for v in z])
        return Job(gen(), 32)

    def ny1_job():
        def gen():
            zero = jnp.zeros((8, 128), f32)
            t = []
            for n0 in range(4):
                t.append(_fft16_a([(x1[4 * n1 + n0, dyn(512, 8), :], zero) for n1 in range(4)], n0, -1))
                yield token(t[-1][1][0], t[-1][3][1], t[-1][0][0], t[-1][2][0])
            acc = [[zero, zero], [zero, zero]]
            for k0 in range(4):
                o = _radix4([t[n0][k0] for n0 in range(4)], -1)
                for k1 in range(4):
                    k = k0 + 4 * k1
                    v = twid(k, o[k1][0], o[k1][1], -1)
                    acc[k // 8] = [jnp.where(row8 == k % 8, v[e], acc[k // 8][e]) for e in range(2)]
                yield token(*acc[0], *acc[1])
            yield put3(lf, 0, *acc)
        return Job(gen(), 9)

    def ny_f():
        (xr, xi), = cdft(lf, 8, False)
        wr_ = _bf(wtr[0, dyn(256, 8), :]).astype(f32)
        wi_ = _bf(wti[0, dyn(256, 8), :]).astype(f32)
        yr, yi = cmul(xr, xi, wr_, wi_)
        put3(li, 0, (yr[0:8], yi[0:8]), (yr[8:16], yi[8:16]))

    def ny_i():
        (dr, di), = cdft(li, 8, True)
        do[0, 0:16, :] = dr
        do[1, 0:16, :] = di

    def ny3_job():
        def gen():
            t = []
            for n0 in range(4):
                a4 = []
                for n1 in range(4):
                    k = 4 * n1 + n0
                    re, im = (jnp.broadcast_to(do[e, pl.ds(zr[0] + k, 1), :], (8, 128)) for e in range(2))
                    a4.append(twid(k, re, im, +1))
                t.append(_fft16_a(a4, n0, +1))
                yield token(t[-1][1][0], t[-1][3][1], t[-1][0][0], t[-1][2][1])
            for k0 in range(4):
                o = _radix4([t[n0][k0] for n0 in range(4)], +1)
                for k1 in range(4):
                    nyb[k0 + 4 * k1] = o[k1][0]
                yield token(*[o[k1][0] for k1 in range(4)])
        return Job(gen(), 8)

    def si_tile(j, fused):
        def yk(r):
            return yp[j // 2, dyn(r, 64), (j % 2) * 128:(j % 2 + 1) * 128]

        e0 = _dot(_bf(yk(0)), _bf(cb[328:392, 0:128]), _TN)
        e2 = _dot(_bf(yk(128)), _bf(cb[328:392, 128:256]), _TN)
        y13 = jnp.concatenate([yk(64), yk(192)], axis=0)
        pq = _dot(_bf(y13), _bf(cb[200:328, :]), _TN)
        p, q = pq[:, 0:128], pq[:, 128:256]
        ep, em = e0 + e2, e0 - e2
        sync[0] = None
        st = jnp.concatenate([ep + p, em + q, ep - p, em - q], axis=1)
        rs = slice(j * 128, (j + 1) * 128)
        if fused:
            ob[rs, :] = (xb[rs, :].astype(f32) + st * gate[dyn(j * 128, 128), :]).astype(jnp.bfloat16)
        else:
            sbuf[j // 4] = st

    d0, d1 = dyn(0, MQ, 0), dyn(0, MQ, 1)

    def strassen(prod, bufs, out):
        put, get = bufs
        put(0, prod(0))
        yield
        m = prod(1)
        put(1, m)
        put(2, get(0, 0) - m)
        yield
        m = prod(2)
        put(3, m)
        put(4, get(2, 0) + m)
        yield
        out(1, 1, prod(3) + get(4, 0))
        yield
        m = prod(4)
        out(0, 1, get(3, 0) + m)
        put(5, get(0, 1) - m)
        yield
        m = prod(5)
        out(1, 0, get(1, 0) + m)
        put(6, get(5, 0) + m)
        yield
        out(0, 0, prod(6) + get(6, 0))
        yield

    def g_quad(q, jobs, after):
        cur = [0]
        vb_ = (va, vb, vc, vd, ve, vf, vg)
        ub_ = (ua, ub, uc, ud, ue, uf, ug)

        def prod(n, m):
            o = 7 * n + m
            lhs = jnp.concatenate(
                [sa[kt, o // 2, dyn(0, MQ // 2), (o % 2) * 128:(o % 2 + 1) * 128] for kt in range(4)], axis=1)
            if n in _RDIR and m in _RDIR:
                kq, tn = 2 * _RDIR[n][0] + _RDIR[m][0], 2 * _RDIR[n][1] + _RDIR[m][1]
                w = wspb[pl.ds(blk(q, 128, tn * KQ), 128), kq * KQ:(kq + 1) * KQ]
            else:
                t, ix = tslot(n, m)
                w = _bf(t[ix, dyn(0, 64), :])
            tk = spread(jobs.get(cur[0], []), 22)
            r = _dot(_bf(synced(lhs)), w, _NT)
            sync[0] = token(r[MQ - SYL:MQ - SYL + 8])
            return tiev(r, tk)

        def vput(k, v):
            vb_[k][0:MQ, :] = v

        def vget(k, w):
            return vb_[k][d1 if w else d0, :]

        def emit(half, tile, m2, tn, c):
            tq = tn + 2 * tile
            j = q + 4 * tq
            lo = half * MH + m2 * MQ
            n = min(MQ, FH - lo)
            hv = gelu2(y1s[j, dyn(lo, n), :]) * (c[0:n] + bbc[j, dyn(0, 8), :][0:1])
            h, hl = hlanes(tq)
            h[lo // 2:(lo + n) // 2, hl] = _pk(hv)

        def combine(n, m2, tn, m):
            s = 2 * m2 + tn

            def put(k, v):
                ub_[k][s, 0:MQ, :] = v

            def get(k, w):
                return ub_[k][s, d1 if w else d0, :]

            if n == 0:
                put(0, m)
            elif n == 1:
                put(1, m)
                put(2, get(0, 0) - m)
            elif n == 2:
                put(3, m)
                put(4, get(2, 0) + m)
            elif n == 3:
                emit(1, 1, m2, tn, m + get(4, 0))
            elif n == 4:
                emit(0, 1, m2, tn, get(3, 0) + m)
                put(5, get(0, 1) - m)
            elif n == 5:
                emit(1, 0, m2, tn, get(1, 0) + m)
                put(6, get(5, 0) + m)
            else:
                emit(0, 0, m2, tn, m + get(6, 0))

        for n in range(7):
            for _ in strassen(lambda m, n=n: prod(n, m), (vput, vget),
                              lambda i, j, v, n=n: combine(n, i, j, v)):
                for fn in after.get(cur[0], []):
                    fn()
                cur[0] += 1

    def tjobs(jobs, q, last=False):
        over(jobs, tprep_job(q, 1), 0, 27)
        if not last:
            over(jobs, tprep_job(q + 1, 0), 29, 49)

    jobs, after = {}, {}
    Q0 = CFG["q0"]
    over(jobs, wout_job(), *Q0["wo"])
    over(jobs, wprep_a_job(), *Q0["wa"])
    over(jobs, wprep_b_job(), *Q0["wb"])
    tjobs(jobs, 0)
    over(jobs, ny1_job(), *Q0["s1"])
    add(after, Q0["f"], ny_f)
    add(after, Q0["i"], ny_i)
    over(jobs, ny3_job(), *Q0["s3"])
    add(after, 37, lambda: o_tile(0, 2, False))
    add(after, 41, lambda: o_tile(0, 3, False))
    g_quad(0, jobs, after)
    wait(grp_4)

    def p2_body(it, carry):
        sync[0] = None
        q = 1 + it
        jobs, after = {}, {}
        for c in range(4):
            a1, b1, a3, b3 = CFG["fs"][c]
            over(jobs, s1_job(c, it), a1, b1 + 1)
            add(after, CFG["tf"][c], lambda c=c: f_op(c, it))
            add(after, CFG["tf"][c] + 3, i_op)
            over(jobs, s3_job(c, it), a3, b3 + 1)
        tjobs(jobs, q)
        add(after, 2, lambda: o_tile(q - 1, 0, False))
        add(after, 6, lambda: o_tile(q - 1, 1, False))
        add(after, 38, lambda: o_tile(q, 2, False))
        add(after, 43, lambda: o_tile(q, 3, False))
        g_quad(q, jobs, after)
        return carry

    jax.lax.fori_loop(0, 2, p2_body, 0)
    sync[0] = None

    outs = []

    def out_dma(lo, hi, bases=(0, 4, 8, 12)):
        for base in bases:
            outs.append(o_cp(base + lo, base + hi))
            outs[-1].start()

    jobs, after = {}, {}
    tjobs(jobs, 3, last=True)
    add(after, 2, lambda: o_tile(2, 0, False))
    add(after, 5, lambda: o_tile(2, 1, False))
    gated = [j for j in range(NB) if j % 4 != 3]
    for n in range(6):
        add(after, 7 + 3 * n, lambda n=n: (si_tile(gated[2 * n], True), si_tile(gated[2 * n + 1], True)))
    add(after, 26, lambda: (si_tile(3, False), si_tile(7, False)))
    add(after, 29, lambda: (si_tile(11, False), si_tile(15, False)))
    add(after, 31, lambda: out_dma(0, 3))
    add(after, 43, lambda: o_tile(3, 2, True))
    add(after, 48, lambda: o_tile(3, 3, True))
    g_quad(3, jobs, after)
    o_tile(3, 0, True)
    out_dma(3, 4, (8, 12))
    o_tile(3, 1, True)
    out_dma(3, 4, (0,))
    out_dma(3, 4, (4,))
    wait(outs)


@jax.jit
def pallas_recurrent_scan__spectral_gfnet__mixer_gmlp__prompt_kernel(
    A_x: jax.Array,
    A_w_r: jax.Array,
    A_w_i: jax.Array,
    B_x: jax.Array,
    B_w_in: jax.Array,
    B_w_sp: jax.Array,
    B_b_sp: jax.Array,
    B_w_out: jax.Array,
):
    del B_x
    bf16, f32, u32 = jnp.bfloat16, jnp.float32, jnp.uint32
    hbm_spec = pl.BlockSpec(memory_space=pltpu.HBM)
    scratch = [
        pltpu.VMEM((S, D), bf16),
        pltpu.VMEM((F, D), bf16),
        pltpu.VMEM((F // 2, D), u32),
        pltpu.VMEM((FH, D), bf16),
        pltpu.VMEM((FHP // 2, D), u32),
        pltpu.VMEM((S, S), bf16),
        pltpu.VMEM((4 * S,), bf16),
        pltpu.VMEM((NB, 32, 128), f32),
        pltpu.VMEM((257, S), bf16),
        pltpu.VMEM((257, S), bf16),
        pltpu.VMEM((2, S // 2, 128), u32),
        pltpu.VMEM((2, S // 2, 128), u32),
        pltpu.VMEM((S // 2, 128), u32),
        pltpu.VMEM((8, 264, 128), u32),
        pltpu.VMEM((8, 264, 128), u32),
        pltpu.VMEM((528, 256), u32),
        pltpu.VMEM(_TW.shape, f32),
        pltpu.VMEM((9, 64, 256), u32),
        pltpu.VMEM((9, 64, 256), u32),
        pltpu.VMEM((7, MH // 2, 256), u32),
    ] + [pltpu.VMEM((MH, 128), f32)] * 10 + [
    ] + [pltpu.VMEM((64, 768), u32)] * 4 + [
        pltpu.VMEM((2, 256, 128), f32),
        pltpu.VMEM((2, 256, 128), f32),
        pltpu.VMEM((32, 128), f32),
        pltpu.VMEM((32, 128), f32),
        pltpu.VMEM((NB, 544, 128), f32),
        pltpu.VMEM((NB, 2 * MH, 128), f32),
    ] + [pltpu.VMEM((2 * MH, 128), f32)] * 4 + [
        pltpu.VMEM((7, MH, 128), f32),
        pltpu.VMEM((4, 25, 96, 256), u32),
        pltpu.VMEM((28, 64, KQ), u32),
        pltpu.VMEM((21, 64, KQ), u32),
    ] + [pltpu.VMEM((4, 192, 128), f32)] * 7 + [
    ] + [pltpu.VMEM((192, 128), f32)] * 7 + [
    ] + [
        pltpu.VMEM((MH, 256), u32),
        pltpu.VMEM((MH, 256), u32),
        pltpu.VMEM((256, 384), u32),
        pltpu.VMEM((256, 384), u32),
        pltpu.VMEM((2, 512, 128), f32),
        pltpu.VMEM((NB, 8, 128), f32),
        pltpu.VMEM((NB // 2, 256, 256), u32),
        pltpu.VMEM((S, D), f32),
        pltpu.VMEM((4, 128, D), f32),
        pltpu.VMEM((S, D), bf16),
        pltpu.SMEM((8,), jnp.int32),
        pltpu.SemaphoreType.DMA((11,)),
    ]
    return pl.pallas_call(
        _kernel,
        in_specs=[hbm_spec] * 10,
        out_specs=hbm_spec,
        out_shape=jax.ShapeDtypeStruct(A_x.shape, A_x.dtype),
        scratch_shapes=scratch,
        compiler_params=pltpu.CompilerParams(vmem_limit_bytes=110 * 1024 * 1024),
    )(A_x, A_w_r.T, A_w_i.T, B_w_in.T, B_w_sp, B_b_sp, B_w_out, jnp.asarray(_CB), jnp.asarray(_TW),
      jnp.asarray(np.zeros((8,), np.int32)))
```
